```python
import jax
import jax.numpy as jnp

def _softmax(x, axis=-1):
    return jax.nn.softmax(x, axis=axis)
def _gelu(x):
    return jax.nn.gelu(x, approximate=True)
def _silu(x):
    return jax.nn.silu(x)
def _sigmoid(x):
    return jax.nn.sigmoid(x)
def _layernorm(x, axis=-1, eps=1e-5):
    m = jnp.mean(x, axis=axis, keepdims=True)
    v = jnp.var(x, axis=axis, keepdims=True)
    return (x - m) / jnp.sqrt(v + eps)
def _scatter_add(tgt, idx, src, axis=0):
    return tgt.at[idx].add(src)
def _segment_sum(src, seg, n):
    return jax.ops.segment_sum(src, seg, n)
class _Rng:
    def __init__(self, key):
        self._k = key
    def _next(self):
        self._k, sub = jax.random.split(self._k)
        return sub
    def normal(self, shape):
        return jax.random.normal(self._next(), shape, dtype=jnp.bfloat16)
    def randint(self, lo, hi, shape):
        return jax.random.randint(self._next(), shape, lo, hi, dtype=jnp.int32)
    def uniform(self, shape, lo=0.0, hi=1.0):
        return jax.random.uniform(self._next(), shape, jnp.bfloat16, lo, hi)
    def permutation(self, n):
        return jax.random.permutation(self._next(), n)


kernel_name = 'parallel_sum__ssm_conv_h3__dense_activation_gelu__prompt'

def setup_inputs():
    _rng = _Rng(jax.random.key(int.from_bytes(__import__("os").urandom(4), "little")))
    _w = (lambda a: (lambda t: t.astype(jnp.bfloat16) if jnp.issubdtype(t.dtype, jnp.floating) else t)(jnp.asarray(a)))
    def _A_setup():
        B, S, D = 1, 2048, 640
        ks = 4
        return {
            "q": _w((lambda *s: _rng.normal(s) * 0.05)(B, S, D)),
            "k": _w((lambda *s: _rng.normal(s) * 0.05)(B, S, D)),
            "v": _w((lambda *s: _rng.normal(s) * 0.05)(B, S, D)),
            "shift_k": _w((lambda *s: _rng.normal(s) * 0.05)(D, ks) * 0.5),
            "ssm_k": _w((lambda *s: _rng.normal(s) * 0.05)(D, S) * (1.0 / S ** 0.5)),
            "ssm_D": _w((lambda *s: _rng.normal(s) * 0.05)(D)),
        }
    _A_in = _A_setup()

    def _B_setup():
        B, S, D, F = 1, 2048, 640, 1728
        return {
            "x": _w((lambda *s: _rng.normal(s) * 0.05)(B, S, D)),
            "w1": _w((lambda *s: _rng.normal(s) * 0.05)(D, F) * (D ** -0.5)),
            "b1": _w((lambda *s: _rng.normal(s) * 0.05)(F) * 0.01),
            "w2": _w((lambda *s: _rng.normal(s) * 0.05)(F, D) * (F ** -0.5)),
            "b2": _w((lambda *s: _rng.normal(s) * 0.05)(D) * 0.01),
        }
    _B_in = _B_setup()

    return {
        "A_q": _A_in["q"],
        "A_k": _A_in["k"],
        "A_v": _A_in["v"],
        "A_shift_k": _A_in["shift_k"],
        "A_ssm_k": _A_in["ssm_k"],
        "A_ssm_D": _A_in["ssm_D"],
        "B_x": _B_in["x"],
        "B_w1": _B_in["w1"],
        "B_b1": _B_in["b1"],
        "B_w2": _B_in["w2"],
        "B_b2": _B_in["b2"],
    }

def reference(A_q, A_k, A_v, A_shift_k, A_ssm_k, A_ssm_D, B_x, B_w1, B_b1, B_w2, B_b2):
    def _A_ref(q, k, v, shift_k, ssm_k, ssm_D):
        B, S, D = q.shape
        ks = shift_k.shape[-1]
        k_pad = jnp.pad(k, ((0, 0), (ks - 1, 0), (0, 0)))
        k_shift = jnp.zeros_like(k)
        for t in range(ks):
            k_shift = k_shift + k_pad[:, t:t + S, :] * shift_k[:, ks - 1 - t][None, None, :]
        kv = k_shift * v
        L = 2 * S
        kv_pad = jnp.pad(kv, ((0, 0), (0, S), (0, 0)))
        kf_pad = jnp.pad(ssm_k, ((0, 0), (0, S)))
        kv_f = (lambda x, axes=(-2,-1): jnp.fft.rfft2(x.astype(jnp.float32), axes=axes))(kv_pad[:, None, :, :], axes=(1, 2))
        kf_f = (lambda x, axes=(-2,-1): jnp.fft.rfft2(x.astype(jnp.float32), axes=axes))(kf_pad[:, None, :], axes=(1, 2))
        kf_f = (lambda x, *d: x.transpose(*d))(kf_f, 1, 2, 0)
        y_f = kv_f * kf_f[None, :, :, :]
        y = (lambda x, s, axes=(-2,-1): jnp.fft.irfft2(x, s=s, axes=axes).astype(jnp.bfloat16))(y_f, (1, L), axes=(1, 2))[:, 0, :S, :]
        y = y + kv * ssm_D[None, None, :]
        return q * y

    def _B_ref(x, w1, b1, w2, b2):
        h = jnp.einsum("bsd,df->bsf", x, w1) + b1
        h = _gelu(h)
        return jnp.einsum("bsf,fd->bsd", h, w2) + b2

    x = A_q
    xn = _layernorm(x, axis=-1)
    return x + _A_ref(xn, A_k, A_v, A_shift_k, A_ssm_k, A_ssm_D) + _B_ref(xn, B_w1, B_b1, B_w2, B_b2)
```

```python
import functools
import itertools
import jax
import jax.numpy as jnp
import numpy as np
from jax import lax
import jax.experimental.pallas as pl
import jax.experimental.pallas.tpu as pltpu

T = 128
C = 128
Q = C // 2
R = 256
NC = R // C
FC = 512
HALO = 8
PIECE = 8
KVR = 32
LNR = 32
VARIANTS = (
    (0, 0, 2, 3, 0.15, 0.85, False),
    (1, 3, 2, 3, 0.15, 0.85, False),
    (4, 5, 2, 3, 0.15, 0.85, False),
    (6, 7, 2, 3, 0.15, 0.95, True),
)

_NT = (((1,), (1,)), ((), ()))
_F32 = jnp.float32
_BF16 = jnp.bfloat16
_U32 = jnp.uint32


def _dft_tables():
    i = np.arange(C)
    f = np.where(i < Q, 2 * i, 2 * (i - Q) + 1)
    ang = np.pi * (2 * f[:, None] + 1) * i[None, :] / (2 * C)
    both = np.stack([np.cos(ang), -np.sin(ang)])
    fwd = both.reshape(2, C // PIECE, PIECE, C).transpose(1, 0, 2, 3).reshape(2 * C, C)
    fwd_kv = fwd[:, (i >> 1) + (i & 1) * Q]
    inv = both.transpose(2, 1, 0).reshape(C, 2 * C) * (2.0 / C)

    def words(m):
        u = np.ascontiguousarray(m, np.float32).view(np.uint32)
        u = (u + 0x7FFF + ((u >> 16) & 1)) >> 16
        return (u[0::2] | (u[1::2] << 16)).astype(np.uint32)

    inv = words(inv)
    return np.concatenate([words(fwd), words(fwd_kv), inv[:, :T], inv[:, T:]]).reshape(6, Q, T)


_TABLES = _dft_tables()


def _pack(even, odd):
    return pltpu.pack_elementwise([even, odd], packed_dtype=_BF16)


def _unpack(x):
    return pltpu.bitcast(x, _BF16)


def _kernel(q_hbm, k_hbm, v_hbm, sk_hbm, h_hbm, d_hbm, w1_hbm, b1_hbm, w2_hbm, b2_hbm, tab_hbm, o_ref,
            q_ref, k_ref, v_ref, h_ref, w1_ref, w2_ref, tab_ref, sk_ref, d_ref, b1_ref, b2_ref,
            blk_sems, w_sems, small_sems,
            vec_ref, b1v_ref, kbuf, xs, hs, kprev, xn_ref, xnb_ref, kvb_ref, mix_ref, *, nsteps):
    step = pl.program_id(0)
    D = k_hbm.shape[-1]
    Fdim = w1_hbm.shape[0]
    ks = sk_hbm.shape[0]
    nd = D // T
    nf = pl.cdiv(Fdim, T)
    nsl = pl.cdiv(Fdim, FC)
    npc = C // PIECE
    nchunks = nsteps * NC

    def tile(i):
        return slice(i * T, min((i + 1) * T, Fdim))

    def rows_of(s):
        return pl.ds(s * R, R) if isinstance(s, int) else pl.ds(pl.multiple_of(s * R, R), R)

    def q_copy(s):
        return [pltpu.make_async_copy(q_hbm.at[0, rows_of(s)], q_ref.at[s % 3], blk_sems.at[0, s % 2])]

    def kvh_copies(s):
        return [pltpu.make_async_copy(h_hbm.at[:, rows_of(s)], h_ref.at[s % 2], blk_sems.at[1, s % 2]),
                pltpu.make_async_copy(k_hbm.at[0, rows_of(s)], k_ref.at[s % 2], blk_sems.at[2, s % 2]),
                pltpu.make_async_copy(v_hbm.at[0, rows_of(s)], v_ref.at[s % 2], blk_sems.at[3, s % 2])]

    def weight_copies(which, j):
        rows = pl.ds(j * FC, min(FC, Fdim - j * FC))
        src, dst = ((w1_hbm, w1_ref), (w2_hbm, w2_ref))[which]
        return [pltpu.make_async_copy(src.at[rows, tile(l)], dst.bitcast(_BF16).at[l, rows],
                                      w_sems.at[which, j]) for l in range(nd)]

    def small_copies():
        pairs = ((tab_hbm, tab_ref), (sk_hbm, sk_ref), (d_hbm, d_ref), (b1_hbm, b1_ref), (b2_hbm, b2_ref))
        return [pltpu.make_async_copy(a, b, small_sems.at[i]) for i, (a, b) in enumerate(pairs)]

    def start(copies):
        for cp in copies:
            cp.start()

    def wait(copies):
        for cp in copies:
            cp.wait()

    def weight_tile(ref, l, j):
        return _unpack(ref[l, tile(j).start // 2:tile(j).stop // 2, :])

    def layer_norm(s, i):
        rows = slice(i * LNR, (i + 1) * LNR)
        x = q_ref[s % 3, rows, :].astype(_F32)
        mu = jnp.mean(x, axis=-1, keepdims=True)
        yield 6 * LNR // 8
        xc = x - mu
        var = jnp.mean(xc * xc, axis=-1, keepdims=True)
        yield 14 * LNR // 8
        xn = xc * lax.rsqrt(var + 1e-5)
        for l in range(nd):
            xn_ref[s % 2, l, rows, :] = xn[:, tile(l)]
        yield 6 * LNR // 8
        n = LNR // 4
        at = (i * LNR // C) * Q + (i * LNR % C) // 4
        for l in range(nd):
            part = [xn_ref[s % 2, l, pl.ds(i * LNR + j, n, stride=4), :] for j in range(4)]
            xnb_ref[s % 2, l, at:at + n, :] = _pack(part[0], part[2])
            xnb_ref[s % 2, l, C // 4 + at:C // 4 + at + n, :] = _pack(part[1], part[3])
        yield 4 * LNR // 8

    @pl.when(step == 0)
    def _():
        start(q_copy(0) + weight_copies(0, 0) + small_copies() + kvh_copies(0))
        wait(q_copy(0))
        for i in range(R // LNR):
            for _ in layer_norm(0, i):
                pass
        start(weight_copies(0, 1))
        wait(small_copies())
        vec_ref[0:ks, :] = sk_ref[...].astype(_F32)
        vec_ref[ks:ks + 1, :] = d_ref[...].astype(_F32)[None, :]
        vec_ref[ks + 1:ks + 2, :] = 2.0 * b2_ref[...].astype(_F32)[None, :]
        b1v_ref[0:1, :] = b1_ref[...].astype(_F32)[None, :]
        kbuf[:, 0:HALO, :] = jnp.zeros((nd, HALO, T), _F32)

    @pl.when(step > 0)
    def _():
        wait(kvh_copies(step))

        @pl.when(step + 1 < nsteps)
        def _():
            wait(q_copy(step + 1))
            start(kvh_copies(step + 1))

        @pl.when(step + 2 < nsteps)
        def _():
            start(q_copy(step + 2))

    def body(first_step, last_step, w_in, w_out, w_kv, span, late):
        first = first_step == 0
        slot = step % 2
        p0 = step * NC
        nq = (last_step + 1) * NC
        sure = (first_step + 1) * NC
        za, zb, zh = step >> 12, step >> 13, step >> 14
        zo = [step >> (15 + l) for l in range(nd)]

        def gated_kv(l):
            lanes = tile(l)
            for c in range(NC):
                rows = slice(c * C, (c + 1) * C)
                kbuf[l, HALO + c * C:HALO + (c + 1) * C, :] = k_ref[slot, rows, lanes].astype(_F32)
            for c in range(NC):
                for r in range(0, Q, KVR):
                    halves = []
                    for lo in (c * C + r, c * C + Q + r):
                        ksh = None
                        for j in range(ks):
                            t = kbuf[l, HALO - j + lo:HALO - j + lo + KVR, :] * vec_ref[j:j + 1, lanes]
                            ksh = t if ksh is None else ksh + t
                        halves.append(ksh * v_ref[slot, lo:lo + KVR, lanes].astype(_F32))
                    kvb_ref[c, l, r:r + KVR, :] = _pack(*halves)
                    yield int(w_kv * vpu_total / (nd * NC * Q // KVR))
            kbuf[l, 0:HALO, :] = kbuf[l, R:R + HALO, :]

        def forward(l):
            for half in range(2):
                kk = [lax.dot_general(_unpack(tab_ref[half]), h_ref[slot, tile(l), c * C:(c + 1) * C], _NT,
                                      preferred_element_type=_F32) for c in range(NC)]
                for j in range(npc // 2):
                    i = half * npc // 2 + j
                    prev = None if first else (kprev[l, 16 * i:16 * i + 8], kprev[l, 16 * i + 8:16 * i + 16])
                    for c in range(NC):
                        re, im = kk[c][16 * j:16 * j + 8], kk[c][16 * j + 8:16 * j + 16]
                        if prev is None:
                            re = re + vec_ref[ks:ks + 1, tile(l)]
                            hc, hd = re, im
                        elif half == 0:
                            hc, hd = re - prev[1], im + prev[0]
                        else:
                            hc, hd = re + prev[1], im - prev[0]
                        hs[l, i, p0 + c, 0:8] = hc
                        hs[l, i, p0 + c, 8:16] = hd - hc
                        hs[l, i, p0 + c, 16:24] = hd + hc
                        prev = re, im
                    kprev[l, 16 * i:16 * i + 8] = prev[0]
                    kprev[l, 16 * i + 8:16 * i + 16] = prev[1]
                yield NC
            for c in range(NC):
                for half in range(2):
                    x = jnp.dot(_unpack(tab_ref[2 + half]), _unpack(kvb_ref[c, l]), preferred_element_type=_F32)
                    for j in range(npc // 2):
                        xs[l, half * npc // 2 + j, p0 + c] = x[16 * j:16 * j + 16]
                yield 2
            ready.add(l)

        xi = [p0 + NC - 1 - e if e < sure else jnp.where(p0 + NC - 1 >= e, p0 + NC - 1 - e, nchunks)
              for e in range(nq)]
        hi = [m if m < sure else jnp.where(m < p0 + NC, m, nchunks) for m in range(nq)]
        held = []

        def mac(l, i):
            xv = {}
            cost = 0
            acc = [None] * NC
            for m in reversed(range(nq)):
                hk = [hs[l, i, hi[m], j * PIECE:(j + 1) * PIECE] for j in range(3)]
                for c in range(NC):
                    e = m + NC - 1 - c
                    if e >= nq:
                        continue
                    if e not in xv:
                        a, b = xs[l, i, xi[e], 0:PIECE], xs[l, i, xi[e], PIECE:2 * PIECE]
                        xv[e] = (a + b, a, b)
                    new = [x * h for x, h in zip(xv[e], hk)]
                    acc[c] = new if acc[c] is None else [s + t for s, t in zip(acc[c], new)]
                    cost += 6
                cost += 1
                if m % 2 == 0:
                    if held:
                        hs[l, i, zh + nchunks + 1, 0:PIECE] = held.pop()
                    held.append(acc[NC - 1][2])
                if m % 1 == 0:
                    yield cost
                    cost = 0
            for c in range(NC):
                s1, s2, s3 = acc[c]
                mix_ref[za + nf + c * nd + l, i * PIECE:(i + 1) * PIECE, :] = _pack(s1 - s3, s1 + s2)
            yield 3 * NC

        def vpu_stream():
            nln = R // LNR
            if first:
                yield "pause"
                wait(kvh_copies(0))
            for l in range(nd):
                yield from gated_kv(l)
                yield "kv%d" % l
            for l in range(nd):
                yield "wait%d" % l
                for i in range(npc):
                    yield from mac(l, i)
                    if first:
                        xs[l, i, nchunks] = jnp.zeros((2 * PIECE, T), _F32)
                        hs[l, i, nchunks] = jnp.zeros((3 * PIECE, T), _F32)
                    k = l * npc + i
                    for t in range(k * nln // (nd * npc), (k + 1) * nln // (nd * npc)):
                        if first and t == 0:
                            assert "q1" in marks
                            wait(q_copy(1))
                        yield from layer_norm(step + 1, t)
                yield "mac%d" % l

        vpu_total = 30 * R // 8 + nd * npc * (6 * (NC * nq - NC * (NC - 1) // 2) + nq + 3 * NC)

        def mlp_in(j, c, defer=None):
            fl = tile(j)
            if first and c == 0 and j % (FC // T) == 0:
                n = j // (FC // T)
                wait(weight_copies(0, n))
                if n == 0:
                    start(q_copy(1))
                    marks.add("q1")
                if n + 2 < nsl:
                    start(weight_copies(0, n + 2))
                elif n + 2 == nsl:
                    start(weight_copies(1, 0) + weight_copies(1, 1))
                else:
                    for m in range(2, nsl):
                        start(weight_copies(1, m))
            h = b1v_ref[0:1, fl]
            for kt in range(nd):
                h = h + lax.dot_general(_unpack(xnb_ref[slot, kt, c * Q:(c + 1) * Q, :]),
                                        weight_tile(w1_ref, kt, j), _NT, preferred_element_type=_F32)
                if kt < nd - 1:
                    yield w_in
            inner = h * (0.7978845608028654 + 0.035677408136300125 * (h * h))
            act = h * (1.0 + jnp.tanh(inner))
            act = _pack(act[0:Q], act[Q:C])

            def store():
                mix_ref[zb + j, c * Q:(c + 1) * Q, 0:fl.stop - fl.start] = act

            if defer is None:
                store()
            else:
                defer.append(store)
            yield w_in

        hist = []

        def gated_conv(l, c):
            g = jnp.concatenate([tab_ref[4], tab_ref[5]], axis=1)
            y2 = jnp.dot(_unpack(g), _unpack(mix_ref[za + nf + c * nd + l]), preferred_element_type=_F32)
            return xn_ref[slot, l, c * C:(c + 1) * C, :] * y2 + vec_ref[ks + 1:ks + 2, tile(l)]

        def finish(l, c, acc):
            rows, lanes = slice(c * C, (c + 1) * C), tile(l)
            o_ref[rows, lanes] = (0.5 * acc + q_ref[step % 3, rows, lanes].astype(_F32)).astype(o_ref.dtype)

        def mlp_out(l, c, defer):
            acc = None
            if not late:
                yield "mac%d" % l
                acc = gated_conv(l, c)
                yield 2
            for j in range(nf):
                act = mix_ref[zo[l] + j, c * Q:(c + 1) * Q, 0:tile(j).stop - tile(j).start]
                part = jnp.dot(_unpack(act), weight_tile(w2_ref, l, j), preferred_element_type=_F32)
                acc = part if acc is None else acc + part
                hist.append(acc[0:8])
                if len(hist) > 8 and len(hist) % 4 == 0:
                    mix_ref[za + nf + NC * nd, 0:8] = pltpu.bitcast(hist[-9], _U32)
                if j == 6:
                    while defer:
                        defer.pop()()
                yield w_out
            if late:
                yield "mac%d" % l
                acc = acc + gated_conv(l, c)
            finish(l, c, acc)
            if late:
                yield 2

        def mlp_stream():
            defer = []
            for j in range(nf):
                for c in range(NC):
                    yield from mlp_in(j, c, defer if (j, c) == (nf - 1, NC - 1) else None)
            if first:
                for j in range(nsl):
                    wait(weight_copies(1, j))
                start(kvh_copies(1) + q_copy(2))
            for l in range(nd):
                for c in range(NC):
                    yield from mlp_out(l, c, defer)

        mxu_total = span * (NC * nf * nd * (w_in + w_out) + NC * 6 * nd)
        vpu, mlp = vpu_stream(), mlp_stream()
        marks, ready = set(), set()
        st = dict(n=0, done=0, seen=0, side=None, blocked=None, pause=0)

        def mxu_tick():
            st["n"] += 1
            if st["side"] is not None and st["n"] % 1 == 0:
                item = next(st["side"], None)
                if item is not None:
                    return item
                st["side"] = None
            item = next(mlp, None)
            while isinstance(item, str):
                while item not in marks:
                    if not vpu_tick():
                        for _ in st["side"]:
                            pass
                item = next(mlp, None)
            return item

        def vpu_tick():
            if st["n"] < st["pause"]:
                return False
            if st["blocked"] is not None:
                if st["blocked"] not in ready:
                    return False
                st["blocked"] = None
            got = next(vpu, None)
            if got is None:
                return False
            if not isinstance(got, str):
                st["done"] += got
            elif got == "pause":
                st["pause"] = 20
            elif got.startswith("kv"):
                st["side"] = itertools.chain(st["side"] or (), forward(int(got[2:])))
            elif got.startswith("wait"):
                st["blocked"] = int(got[4:])
            else:
                marks.add(got)
            return True

        while True:
            item = mxu_tick()
            if item is None:
                break
            st["seen"] += item
            while st["done"] * mxu_total < st["seen"] * vpu_total * (1 + w_kv) and vpu_tick():
                pass
        while vpu_tick():
            pass

    for variant in VARIANTS:
        pl.when((step >= variant[0]) & (step <= variant[1]))(functools.partial(body, *variant))


@jax.jit
def pallas_parallel_sum__ssm_conv_h3__dense_activation_gelu__prompt_kernel(
    A_q: jax.Array,
    A_k: jax.Array,
    A_v: jax.Array,
    A_shift_k: jax.Array,
    A_ssm_k: jax.Array,
    A_ssm_D: jax.Array,
    B_x: jax.Array,
    B_w1: jax.Array,
    B_b1: jax.Array,
    B_w2: jax.Array,
    B_b2: jax.Array,
):
    del B_x
    B, S, D = A_q.shape
    Fdim = B_w1.shape[1]
    ks = A_shift_k.shape[1]
    nsteps = S // R
    P = S // C
    nd = D // T
    assert B == 1 and S % R == 0 and D % T == 0 and nsteps == VARIANTS[-1][1] + 1 and ks + 2 <= 8

    args = (A_q, A_k, A_v,
            A_shift_k.T,
            A_ssm_k, A_ssm_D,
            B_w1.T,
            B_b1, B_w2, B_b2, jnp.asarray(_TABLES))
    return pl.pallas_call(
        functools.partial(_kernel, nsteps=nsteps),
        grid=(nsteps,),
        in_specs=[pl.BlockSpec(memory_space=pl.ANY)] * len(args),
        out_specs=pl.BlockSpec((None, R, D), lambda i: (0, i, 0)),
        out_shape=jax.ShapeDtypeStruct((B, S, D), A_q.dtype),
        scratch_shapes=[
            pltpu.VMEM((3, R, D), A_q.dtype),
            pltpu.VMEM((2, R, D), A_k.dtype),
            pltpu.VMEM((2, R, D), A_v.dtype),
            pltpu.VMEM((2, D, R), _BF16),
            pltpu.VMEM((nd, Fdim // 2, T), _U32),
            pltpu.VMEM((nd, Fdim // 2, T), _U32),
            pltpu.VMEM(_TABLES.shape, _U32),
            pltpu.VMEM((ks, D), A_shift_k.dtype),
            pltpu.VMEM((D,), A_ssm_D.dtype),
            pltpu.VMEM((Fdim,), B_b1.dtype),
            pltpu.VMEM((D,), B_b2.dtype),
            pltpu.SemaphoreType.DMA((4, 2)),
            pltpu.SemaphoreType.DMA((2, pl.cdiv(Fdim, FC))),
            pltpu.SemaphoreType.DMA((5,)),
            pltpu.VMEM((8, D), _F32),
            pltpu.VMEM((8, Fdim), _F32),
            pltpu.VMEM((nd, HALO + R, T), _F32),
            pltpu.VMEM((nd, C // PIECE, P + 1, 2 * PIECE, T), _F32),
            pltpu.VMEM((nd, C // PIECE, P + 2, 3 * PIECE, T), _F32),
            pltpu.VMEM((nd, 2 * C, T), _F32),
            pltpu.VMEM((2, nd, R, T), _F32),
            pltpu.VMEM((2, nd, R // 2, T), _U32),
            pltpu.VMEM((NC, nd, Q, T), _U32),
            pltpu.VMEM((pl.cdiv(Fdim, T) + NC * nd + 1, C, T), _U32),
        ],
        compiler_params=pltpu.CompilerParams(
            dimension_semantics=("arbitrary",),
            vmem_limit_bytes=100 * 1024 * 1024,
        ),
    )(*args)
```

```python
import functools
import itertools
import jax
import jax.numpy as jnp
import numpy as np
from jax import lax
import jax.experimental.pallas as pl
import jax.experimental.pallas.tpu as pltpu

T = 128
C = 128
Q = C // 2
R = 256
NC = R // C
W1_CUTS = (0, 2, 5, 9, 14)
HALO = 8
PIECE = 8
KVR = 32
LNR = 32
VARIANTS = (
    (0, 0, 2, 3, 0.3, 1.0, False),
    (1, 3, 2, 3, 0.1, 0.95, True),
    (4, 5, 2, 3, 0.1, 0.95, True),
    (6, 7, 2, 3, 0.1, 0.95, True),
)

_NT = (((1,), (1,)), ((), ()))
_F32 = jnp.float32
_BF16 = jnp.bfloat16
_U32 = jnp.uint32


def _dft_tables():
    i = np.arange(C)
    f = np.where(i < Q, 2 * i, 2 * (i - Q) + 1)
    ang = np.pi * (2 * f[:, None] + 1) * i[None, :] / (2 * C)
    both = np.stack([np.cos(ang), -np.sin(ang)])
    fwd = both.reshape(2, C // PIECE, PIECE, C).transpose(1, 0, 2, 3).reshape(2 * C, C)
    fwd_kv = fwd[:, (i >> 1) + (i & 1) * Q]
    inv = both.transpose(2, 1, 0).reshape(C, 2 * C) * (2.0 / C)

    def words(m):
        u = np.ascontiguousarray(m, np.float32).view(np.uint32)
        u = (u + 0x7FFF + ((u >> 16) & 1)) >> 16
        return (u[0::2] | (u[1::2] << 16)).astype(np.uint32)

    inv = words(inv)
    return np.concatenate([words(fwd), words(fwd_kv), inv[:, :T], inv[:, T:]]).reshape(6, Q, T)


_TABLES = _dft_tables()


def _pack(even, odd):
    return pltpu.pack_elementwise([even, odd], packed_dtype=_BF16)


def _unpack(x):
    return pltpu.bitcast(x, _BF16)


def _kernel(q_hbm, k_hbm, v_hbm, sk_hbm, h_hbm, d_hbm, w1_hbm, b1_hbm, w2_hbm, b2_hbm, tab_hbm, o_ref,
            q_ref, k_ref, v_ref, h_ref, w1_ref, w2_ref, tab_ref, sk_ref, d_ref, b1_ref, b2_ref,
            blk_sems, w_sems, small_sems,
            vec_ref, b1v_ref, kbuf, xs, hs, kprev, xn_ref, xnb_ref, kvb_ref, mix_ref, *, nsteps):
    step = pl.program_id(0)
    D = k_hbm.shape[-1]
    Fdim = w1_hbm.shape[0]
    ks = sk_hbm.shape[0]
    nd = D // T
    nf = pl.cdiv(Fdim, T)
    npc = C // PIECE
    nchunks = nsteps * NC

    def tile(i):
        return slice(i * T, min((i + 1) * T, Fdim))

    def rows_of(s):
        return pl.ds(s * R, R) if isinstance(s, int) else pl.ds(pl.multiple_of(s * R, R), R)

    def q_copy(s):
        return [pltpu.make_async_copy(q_hbm.at[0, rows_of(s)], q_ref.at[s % 3], blk_sems.at[0, s % 2])]

    def kvh_copies(s):
        return [pltpu.make_async_copy(h_hbm.at[:, rows_of(s)], h_ref.at[s % 2], blk_sems.at[1, s % 2]),
                pltpu.make_async_copy(k_hbm.at[0, rows_of(s)], k_ref.at[s % 2], blk_sems.at[2, s % 2]),
                pltpu.make_async_copy(v_hbm.at[0, rows_of(s)], v_ref.at[s % 2], blk_sems.at[3, s % 2])]

    def w1_copies(n):
        rows = pl.ds(W1_CUTS[n] * T, min(W1_CUTS[n + 1] * T, Fdim) - W1_CUTS[n] * T)
        return [pltpu.make_async_copy(w1_hbm.at[rows, tile(l)], w1_ref.bitcast(_BF16).at[l, rows],
                                      w_sems.at[0, n]) for l in range(nd)]

    def w2_copy(l):
        return [pltpu.make_async_copy(w2_hbm.at[:, tile(l)], w2_ref.bitcast(_BF16).at[l], w_sems.at[1, l])]

    def small_copies():
        pairs = ((tab_hbm, tab_ref), (sk_hbm, sk_ref), (d_hbm, d_ref), (b1_hbm, b1_ref), (b2_hbm, b2_ref))
        return [pltpu.make_async_copy(a, b, small_sems.at[i]) for i, (a, b) in enumerate(pairs)]

    def start(copies):
        for cp in copies:
            cp.start()

    def wait(copies):
        for cp in copies:
            cp.wait()

    def weight_tile(ref, l, j):
        return _unpack(ref[l, tile(j).start // 2:tile(j).stop // 2, :])

    def layer_norm(s, i):
        rows = slice(i * LNR, (i + 1) * LNR)
        x = q_ref[s % 3, rows, :].astype(_F32)
        mu = jnp.mean(x, axis=-1, keepdims=True)
        yield 6 * LNR // 8
        xc = x - mu
        var = jnp.mean(xc * xc, axis=-1, keepdims=True)
        yield 14 * LNR // 8
        xn = xc * lax.rsqrt(var + 1e-5)
        for l in range(nd):
            xn_ref[s % 2, l, rows, :] = xn[:, tile(l)]
        yield 6 * LNR // 8
        n = LNR // 4
        at = (i * LNR // C) * Q + (i * LNR % C) // 4
        for l in range(nd):
            if 0 == 0:
                part = [xn_ref[s % 2, l, pl.ds(i * LNR + j, n, stride=4), :] for j in range(4)]
            else:
                part = [xn[j * n:(j + 1) * n, tile(l)] for j in range(4)]
            xnb_ref[s % 2, l, at:at + n, :] = _pack(part[0], part[2])
            xnb_ref[s % 2, l, C // 4 + at:C // 4 + at + n, :] = _pack(part[1], part[3])
        yield 4 * LNR // 8

    def init():
        start(q_copy(0) + small_copies() + w1_copies(0))
        wait(q_copy(0))
        start(w1_copies(1))
        for i in range(R // LNR):
            for _ in layer_norm(0, i):
                pass
        wait(small_copies())
        vec_ref[0:ks, :] = sk_ref[...].astype(_F32)
        vec_ref[ks:ks + 1, :] = d_ref[...].astype(_F32)[None, :]
        vec_ref[ks + 1:ks + 2, :] = 2.0 * b2_ref[...].astype(_F32)[None, :]
        b1v_ref[0:1, :] = b1_ref[...].astype(_F32)[None, :]
        kbuf[:, 0:HALO, :] = jnp.zeros((nd, HALO, T), _F32)

    pl.when(step == 0)(init)

    def refill():
        wait(kvh_copies(step))

        @pl.when(step + 1 < nsteps)
        def _():
            wait(q_copy(step + 1))
            start(kvh_copies(step + 1))

        @pl.when(step + 2 < nsteps)
        def _():
            start(q_copy(step + 2))

    pl.when(step > 0)(refill)

    def body(first_step, last_step, w_in, w_out, w_kv, span, late):
        first = first_step == 0
        slot = step % 2
        p0 = step * NC
        nq = (last_step + 1) * NC
        sure = (first_step + 1) * NC
        za, zb, zh = step >> 12, step >> 13, step >> 14
        zo = [step >> (15 + l) for l in range(nd)]

        def gated_kv(l):
            lanes = tile(l)
            for c in range(NC):
                rows = slice(c * C, (c + 1) * C)
                kbuf[l, HALO + c * C:HALO + (c + 1) * C, :] = k_ref[slot, rows, lanes].astype(_F32)
            for c in range(NC):
                for r in range(0, Q, KVR):
                    halves = []
                    for lo in (c * C + r, c * C + Q + r):
                        ksh = None
                        for j in range(ks):
                            t = kbuf[l, HALO - j + lo:HALO - j + lo + KVR, :] * vec_ref[j:j + 1, lanes]
                            ksh = t if ksh is None else ksh + t
                        halves.append(ksh * v_ref[slot, lo:lo + KVR, lanes].astype(_F32))
                    kvb_ref[c, l, r:r + KVR, :] = _pack(*halves)
                    yield int(w_kv * vpu_total / (nd * NC * Q // KVR))
            kbuf[l, 0:HALO, :] = kbuf[l, R:R + HALO, :]

        def forward(l):
            for half in range(2):
                kk = [lax.dot_general(_unpack(tab_ref[half]), h_ref[slot, tile(l), c * C:(c + 1) * C], _NT,
                                      preferred_element_type=_F32) for c in range(NC)]
                for j in range(npc // 2):
                    i = half * npc // 2 + j
                    prev = None if first else (kprev[l, 16 * i:16 * i + 8], kprev[l, 16 * i + 8:16 * i + 16])
                    for c in range(NC):
                        re, im = kk[c][16 * j:16 * j + 8], kk[c][16 * j + 8:16 * j + 16]
                        if prev is None:
                            re = re + vec_ref[ks:ks + 1, tile(l)]
                            hc, hd = re, im
                        elif half == 0:
                            hc, hd = re - prev[1], im + prev[0]
                        else:
                            hc, hd = re + prev[1], im - prev[0]
                        hs[l, i, p0 + c, 0:8] = hc
                        hs[l, i, p0 + c, 8:16] = hd - hc
                        hs[l, i, p0 + c, 16:24] = hd + hc
                        prev = re, im
                    kprev[l, 16 * i:16 * i + 8] = prev[0]
                    kprev[l, 16 * i + 8:16 * i + 16] = prev[1]
                yield NC
            for c in range(NC):
                for half in range(2):
                    x = jnp.dot(_unpack(tab_ref[2 + half]), _unpack(kvb_ref[c, l]), preferred_element_type=_F32)
                    for j in range(npc // 2):
                        xs[l, half * npc // 2 + j, p0 + c] = x[16 * j:16 * j + 16]
                yield 2
            marks.add(str(l))

        xi = [p0 + NC - 1 - e if e < sure else jnp.where(p0 + NC - 1 >= e, p0 + NC - 1 - e, nchunks)
              for e in range(nq)]
        hi = [m if m < sure else jnp.where(m < p0 + NC, m, nchunks) for m in range(nq)]
        held = []

        def mac(l, i):
            xv = {}
            cost = 0
            acc = [None] * NC
            for m in reversed(range(nq)):
                hk = [hs[l, i, hi[m], j * PIECE:(j + 1) * PIECE] for j in range(3)]
                for c in range(NC):
                    e = m + NC - 1 - c
                    if e >= nq:
                        continue
                    if e not in xv:
                        a, b = xs[l, i, xi[e], 0:PIECE], xs[l, i, xi[e], PIECE:2 * PIECE]
                        xv[e] = (a + b, a, b)
                    new = [x * h for x, h in zip(xv[e], hk)]
                    acc[c] = new if acc[c] is None else [s + t for s, t in zip(acc[c], new)]
                    cost += 6
                cost += 1
                if m % 2 == 0:
                    if held:
                        hs[l, i, zh + nchunks + 1, 0:PIECE] = held.pop()
                    held.append(acc[NC - 1][2])
                if m % 1 == 0:
                    yield cost
                    cost = 0
            for c in range(NC):
                s1, s2, s3 = acc[c]
                mix_ref[za + nf + c * nd + l, i * PIECE:(i + 1) * PIECE, :] = _pack(s1 - s3, s1 + s2)
            yield 3 * NC

        def vpu_stream():
            nln = R // LNR
            if first:
                yield "pause"
                assert "kvh" in marks
                wait(kvh_copies(0))
            for l in range(nd):
                yield from gated_kv(l)
                yield "kv%d" % l
            for l in range(nd):
                yield "wait%d" % l
                for i in range(npc):
                    yield from mac(l, i)
                    if first:
                        xs[l, i, nchunks] = jnp.zeros((2 * PIECE, T), _F32)
                        hs[l, i, nchunks] = jnp.zeros((3 * PIECE, T), _F32)
                        continue
                    k0, k1 = (40, 80)
                    k = min(max(l * npc + i, k0), k1) - k0
                    kn = min(max(l * npc + i + 1, k0), k1) - k0
                    for t in range(k * nln // (k1 - k0), kn * nln // (k1 - k0)):
                        if 1:
                            yield from layer_norm(step + 1, t)
                yield "mac%d" % l
            if first:
                yield "waitq1"
                for t in range(nln):
                    for cost in layer_norm(1, t):
                        yield cost * 3

        vpu_total = 30 * R // 8 + nd * npc * (6 * (NC * nq - NC * (NC - 1) // 2) + nq + 3 * NC)

        def mlp_in(j, c, defer=None):
            fl = tile(j)
            if first and c == 0 and j in W1_CUTS:
                n = W1_CUTS.index(j)
                wait(w1_copies(n))
                if n == 0:
                    start(kvh_copies(0))
                    marks.add("kvh")
                left = len(W1_CUTS) - 2 - n
                start(w1_copies(n + 2) if left > 1 else w2_copy(0) if left else w2_copy(1) + w2_copy(2))
            h = b1v_ref[0:1, fl]
            for kt in range(nd):
                h = h + lax.dot_general(_unpack(xnb_ref[slot, kt, c * Q:(c + 1) * Q, :]),
                                        weight_tile(w1_ref, kt, j), _NT, preferred_element_type=_F32)
                if kt < nd - 1:
                    yield w_in
            inner = h * (0.7978845608028654 + 0.035677408136300125 * (h * h))
            act = h * (1.0 + jnp.tanh(inner))
            act = _pack(act[0:Q], act[Q:C])

            def store():
                mix_ref[zb + j, c * Q:(c + 1) * Q, 0:fl.stop - fl.start] = act

            if defer is None:
                store()
            else:
                defer.append(store)
            yield w_in

        hist = []

        def gated_conv(l, c):
            g = jnp.concatenate([tab_ref[4], tab_ref[5]], axis=1)
            y2 = jnp.dot(_unpack(g), _unpack(mix_ref[za + nf + c * nd + l, 0:C]), preferred_element_type=_F32)
            return xn_ref[slot, l, c * C:(c + 1) * C, :] * y2 + vec_ref[ks + 1:ks + 2, tile(l)]

        def finish(l, c, acc):
            rows, lanes = slice(c * C, (c + 1) * C), tile(l)
            o_ref[rows, lanes] = (0.5 * acc + q_ref[step % 3, rows, lanes].astype(_F32)).astype(o_ref.dtype)

        def mlp_out(l, c, defer):
            acc = None
            if not late:
                yield "mac%d" % l
                acc = gated_conv(l, c)
                yield 2
            for j in range(nf):
                act = mix_ref[zo[l] + j, c * Q:(c + 1) * Q, 0:tile(j).stop - tile(j).start]
                part = jnp.dot(_unpack(act), weight_tile(w2_ref, l, j), preferred_element_type=_F32)
                acc = part if acc is None else acc + part
                hist.append(acc[0:8])
                if len(hist) > 8 and len(hist) % 4 == 0:
                    mix_ref[za + nf + NC * nd, 0:8] = pltpu.bitcast(hist[-9], _U32)
                if j == 6:
                    while defer:
                        defer.pop()()
                yield w_out
            if late:
                yield "mac%d" % l
                acc = acc + gated_conv(l, c)
            finish(l, c, acc)
            if late:
                yield 2

        def mlp_stream():
            defer = []
            for j in range(nf):
                for c in range(NC):
                    yield from mlp_in(j, c, defer if (j, c) == (nf - 1, NC - 1) else None)
            for l in range(nd):
                if first and l == 0:
                    wait(w2_copy(0) + w2_copy(1))
                    start(q_copy(1) + w2_copy(3))
                elif first and l == 2:
                    wait(w2_copy(2) + w2_copy(3) + q_copy(1))
                    marks.add("q1")
                    start(sum((w2_copy(m) for m in range(4, nd)), []) + kvh_copies(1))
                elif first and l >= 4:
                    wait(w2_copy(l))
                    if l == 4:
                        start(q_copy(2))
                for c in range(NC):
                    yield from mlp_out(l, c, defer)

        mxu_total = span * (NC * nf * nd * (w_in + w_out) + NC * 6 * nd)
        vpu, mlp = vpu_stream(), mlp_stream()
        marks = set()
        st = dict(n=0, done=0, seen=0, side=None, blocked=None, pause=0)

        def mxu_tick():
            st["n"] += 1
            if st["side"] is not None and st["n"] % 1 == 0:
                item = next(st["side"], None)
                if item is not None:
                    return item
                st["side"] = None
            item = next(mlp, None)
            while isinstance(item, str):
                while item not in marks:
                    if not vpu_tick():
                        for _ in st["side"]:
                            pass
                item = next(mlp, None)
            return item

        def vpu_tick():
            if st["n"] < st["pause"]:
                return False
            if st["blocked"] is not None:
                if st["blocked"] not in marks:
                    return False
                st["blocked"] = None
            got = next(vpu, None)
            if got is None:
                return False
            if not isinstance(got, str):
                st["done"] += got
            elif got == "pause":
                st["pause"] = 50
            elif got.startswith("kv"):
                st["side"] = itertools.chain(st["side"] or (), forward(int(got[2:])))
            elif got.startswith("wait"):
                st["blocked"] = got[4:]
            else:
                marks.add(got)
            return True

        while True:
            item = mxu_tick()
            if item is None:
                break
            st["seen"] += item
            while st["done"] * mxu_total < st["seen"] * vpu_total * (1 + w_kv) and vpu_tick():
                pass
        while vpu_tick():
            pass

    for variant in VARIANTS:
        pl.when((step >= variant[0]) & (step <= variant[1]))(functools.partial(body, *variant))


@jax.jit
def pallas_parallel_sum__ssm_conv_h3__dense_activation_gelu__prompt_kernel(
    A_q: jax.Array,
    A_k: jax.Array,
    A_v: jax.Array,
    A_shift_k: jax.Array,
    A_ssm_k: jax.Array,
    A_ssm_D: jax.Array,
    B_x: jax.Array,
    B_w1: jax.Array,
    B_b1: jax.Array,
    B_w2: jax.Array,
    B_b2: jax.Array,
):
    del B_x
    B, S, D = A_q.shape
    Fdim = B_w1.shape[1]
    ks = A_shift_k.shape[1]
    nsteps = S // R
    P = S // C
    nd = D // T
    assert B == 1 and S % R == 0 and D % T == 0 and ks + 2 <= 8 and nd > 4 and W1_CUTS[-1] == pl.cdiv(Fdim, T)

    args = (A_q, A_k, A_v,
            A_shift_k.T,
            A_ssm_k, A_ssm_D,
            B_w1.T,
            B_b1, B_w2, B_b2, jnp.asarray(_TABLES))
    return pl.pallas_call(
        functools.partial(_kernel, nsteps=nsteps),
        grid=(nsteps,),
        in_specs=[pl.BlockSpec(memory_space=pl.ANY)] * len(args),
        out_specs=pl.BlockSpec((None, R, D), lambda i: (0, i, 0)),
        out_shape=jax.ShapeDtypeStruct((B, S, D), A_q.dtype),
        scratch_shapes=[
            pltpu.VMEM((3, R, D), A_q.dtype),
            pltpu.VMEM((2, R, D), A_k.dtype),
            pltpu.VMEM((2, R, D), A_v.dtype),
            pltpu.VMEM((2, D, R), _BF16),
            pltpu.VMEM((nd, Fdim // 2, T), _U32),
            pltpu.VMEM((nd, Fdim // 2, T), _U32),
            pltpu.VMEM(_TABLES.shape, _U32),
            pltpu.VMEM((ks, D), A_shift_k.dtype),
            pltpu.VMEM((D,), A_ssm_D.dtype),
            pltpu.VMEM((Fdim,), B_b1.dtype),
            pltpu.VMEM((D,), B_b2.dtype),
            pltpu.SemaphoreType.DMA((4, 2)),
            pltpu.SemaphoreType.DMA((2, max(nd, len(W1_CUTS)))),
            pltpu.SemaphoreType.DMA((5,)),
            pltpu.VMEM((8, D), _F32),
            pltpu.VMEM((8, Fdim), _F32),
            pltpu.VMEM((nd, HALO + R, T), _F32),
            pltpu.VMEM((nd, C // PIECE, P + 1, 2 * PIECE, T), _F32),
            pltpu.VMEM((nd, C // PIECE, P + 2, 3 * PIECE, T), _F32),
            pltpu.VMEM((nd, 2 * C, T), _F32),
            pltpu.VMEM((2, nd, R, T), _F32),
            pltpu.VMEM((2, nd, R // 2, T), _U32),
            pltpu.VMEM((NC, nd, Q, T), _U32),
            pltpu.VMEM((pl.cdiv(Fdim, T) + NC * nd + 1, max(C, R // 2), T), _U32),
        ],
        compiler_params=pltpu.CompilerParams(
            dimension_semantics=("arbitrary",),
            vmem_limit_bytes=100 * 1024 * 1024,
        ),
    )(*args)
```

```python
import functools
import itertools
import jax
import jax.numpy as jnp
import numpy as np
from jax import lax
import jax.experimental.pallas as pl
import jax.experimental.pallas.tpu as pltpu

T = 128
C = 128
Q = C // 2
R = 256
NC = R // C
W1_CUTS = (0, 2, 5, 8, 14)
HALO = 8
PIECE = 8
KVR = 64
LNR = 64
VARIANTS = (
    (0, 0, 2, 3, 0.3, 1.0, False),
    (1, 3, 2, 3, 0.1, 0.95, True),
    (4, 5, 2, 3, 0.1, 0.95, True),
    (6, 7, 2, 3, 0.1, 0.95, True),
)

_NT = (((1,), (1,)), ((), ()))
_F32 = jnp.float32
_BF16 = jnp.bfloat16
_U32 = jnp.uint32


def _dft_tables():
    i = np.arange(C)
    f = np.where(i < Q, 2 * i, 2 * (i - Q) + 1)
    ang = np.pi * (2 * f[:, None] + 1) * i[None, :] / (2 * C)
    both = np.stack([np.cos(ang), -np.sin(ang)])
    fwd = both.reshape(2, C // PIECE, PIECE, C).transpose(1, 0, 2, 3).reshape(2 * C, C)
    inv = fwd.T * (2.0 / C)

    def words(m):
        u = np.ascontiguousarray(m, np.float32).view(np.uint32)
        u = (u + 0x7FFF + ((u >> 16) & 1)) >> 16
        return (u[0::2] | (u[1::2] << 16)).astype(np.uint32)

    inv = words(inv)
    return np.concatenate([words(fwd), inv[:, :T], inv[:, T:]]).reshape(4, Q, T)


_TABLES = _dft_tables()


def _unpack(x):
    return pltpu.bitcast(x, _BF16)


def _load_bf16(ref, lead, rows, cols=slice(None)):
    return _unpack(ref.bitcast(_U32)[(*lead, slice(rows.start // 2, rows.stop // 2), cols)])


def _kernel(q_hbm, k_hbm, v_hbm, sk_hbm, h_hbm, d_hbm, w1_hbm, b1_hbm, w2_hbm, b2_hbm, tab_hbm, o_ref,
            q_ref, k_ref, v_ref, h_ref, w1_ref, w2_ref, tab_ref, sk_ref, d_ref, b1_ref, b2_ref,
            blk_sems, w_sems, small_sems,
            vec_ref, b1v_ref, kbuf, xs, hs, kprev, xn_ref, xnb_ref, kvb_ref, mix_ref, *, nsteps):
    step = pl.program_id(0)
    D = k_hbm.shape[-1]
    Fdim = w1_hbm.shape[0]
    ks = sk_hbm.shape[0]
    nd = D // T
    nf = pl.cdiv(Fdim, T)
    npc = C // PIECE
    nchunks = nsteps * NC

    def tile(i):
        return slice(i * T, min((i + 1) * T, Fdim))

    def chunk(c):
        return slice(c * C, (c + 1) * C)

    def rows_of(s):
        return pl.ds(s * R, R) if isinstance(s, int) else pl.ds(pl.multiple_of(s * R, R), R)

    def q_copy(s):
        return [pltpu.make_async_copy(q_hbm.at[0, rows_of(s)], q_ref.at[s % 3], blk_sems.at[0, s % 2])]

    def kvh_copies(s):
        return [pltpu.make_async_copy(h_hbm.at[:, rows_of(s)], h_ref.at[s % 2], blk_sems.at[1, s % 2]),
                pltpu.make_async_copy(k_hbm.at[0, rows_of(s)], k_ref.at[s % 2], blk_sems.at[2, s % 2]),
                pltpu.make_async_copy(v_hbm.at[0, rows_of(s)], v_ref.at[s % 2], blk_sems.at[3, s % 2])]

    def w1_copies(n):
        rows = pl.ds(W1_CUTS[n] * T, min(W1_CUTS[n + 1] * T, Fdim) - W1_CUTS[n] * T)
        return [pltpu.make_async_copy(w1_hbm.at[rows, tile(l)], w1_ref.at[l, rows],
                                      w_sems.at[0, n]) for l in range(nd)]

    def w2_copy(l):
        return [pltpu.make_async_copy(w2_hbm.at[:, tile(l)], w2_ref.at[l], w_sems.at[1, l])]

    def small_copies():
        pairs = ((tab_hbm, tab_ref), (sk_hbm, sk_ref), (d_hbm, d_ref), (b1_hbm, b1_ref), (b2_hbm, b2_ref))
        return [pltpu.make_async_copy(a, b, small_sems.at[i]) for i, (a, b) in enumerate(pairs)]

    def start(copies):
        for cp in copies:
            cp.start()

    def wait(copies):
        for cp in copies:
            cp.wait()

    def weight_tile(ref, l, j):
        return _load_bf16(ref, (l,), tile(j))

    def layer_norm(s, i):
        rows = slice(i * LNR, (i + 1) * LNR)
        x = q_ref[s % 3, rows, :].astype(_F32)
        mu = jnp.mean(x, axis=-1, keepdims=True)
        yield 6 * LNR // 8
        xc = x - mu
        var = jnp.mean(xc * xc, axis=-1, keepdims=True)
        yield 14 * LNR // 8
        xn = xc * lax.rsqrt(var + 1e-5)
        for l in range(nd):
            xn_ref[s % 2, l, rows, :] = xn[:, tile(l)]
            xnb_ref[s % 2, l, rows, :] = xn[:, tile(l)].astype(_BF16)
        yield 10 * LNR // 8

    def init():
        start(q_copy(0) + small_copies() + w1_copies(0))
        wait(q_copy(0))
        start(w1_copies(1))
        for i in range(R // LNR):
            for _ in layer_norm(0, i):
                pass
        wait(small_copies())
        vec_ref[0:ks, :] = sk_ref[...].astype(_F32)
        vec_ref[ks:ks + 1, :] = d_ref[...].astype(_F32)[None, :]
        vec_ref[ks + 1:ks + 2, :] = 2.0 * b2_ref[...].astype(_F32)[None, :]
        b1v_ref[0:1, :] = b1_ref[...].astype(_F32)[None, :]
        kbuf[:, 0:HALO, :] = jnp.zeros((nd, HALO, T), _F32)

    pl.when(step == 0)(init)

    def body(first_step, last_step, w_in, w_out, w_kv, span, late):
        first = first_step == 0
        slot = step % 2
        p0 = step * NC
        nq = (last_step + 1) * NC
        sure = (first_step + 1) * NC
        za, zb, zh = step >> 12, step >> 13, step >> 14
        zo = [step >> (15 + l) for l in range(nd)]

        def refill():
            if not first:
                start(kvh_copies(step + 1) + q_copy(step + 2))

        if last_step == nsteps - 1:
            wait(kvh_copies(step))

            @pl.when(step < last_step)
            def _():
                wait(q_copy(last_step))
                start(kvh_copies(last_step))
        elif not first:
            wait(kvh_copies(step) + q_copy(step + 1))

        def gated_kv(l):
            lanes = tile(l)
            for c in range(NC):
                rows = slice(c * C, (c + 1) * C)
                kbuf[l, HALO + c * C:HALO + (c + 1) * C, :] = k_ref[slot, rows, lanes].astype(_F32)
            for c in range(NC):
                for r in range(0, C, KVR):
                    lo = c * C + r
                    ksh = None
                    for j in range(ks):
                        t = kbuf[l, HALO - j + lo:HALO - j + lo + KVR, :] * vec_ref[j:j + 1, lanes]
                        ksh = t if ksh is None else ksh + t
                    kv = ksh * v_ref[slot, lo:lo + KVR, lanes].astype(_F32)
                    kvb_ref[l, lo:lo + KVR, :] = kv.astype(_BF16)
                    yield int(w_kv * vpu_total / (nd * R // KVR))
            kbuf[l, 0:HALO, :] = kbuf[l, R:R + HALO, :]

        def forward(l):
            for half in range(2):
                kk = [lax.dot_general(_unpack(tab_ref[half]), h_ref[slot, tile(l), c * C:(c + 1) * C], _NT,
                                      preferred_element_type=_F32) for c in range(NC)]
                for j in range(npc // 2):
                    i = half * npc // 2 + j
                    prev = None if first else (kprev[l, 16 * i:16 * i + 8], kprev[l, 16 * i + 8:16 * i + 16])
                    for c in range(NC):
                        re, im = kk[c][16 * j:16 * j + 8], kk[c][16 * j + 8:16 * j + 16]
                        if prev is None:
                            re = re + vec_ref[ks:ks + 1, tile(l)]
                            hc, hd = re, im
                        elif half == 0:
                            hc, hd = re - prev[1], im + prev[0]
                        else:
                            hc, hd = re + prev[1], im - prev[0]
                        hs[l, i, p0 + c, 0:8] = hc
                        hs[l, i, p0 + c, 8:16] = hd - hc
                        hs[l, i, p0 + c, 16:24] = hd + hc
                        prev = re, im
                    kprev[l, 16 * i:16 * i + 8] = prev[0]
                    kprev[l, 16 * i + 8:16 * i + 16] = prev[1]
                yield NC
            for c in range(NC):
                for half in range(2):
                    x = jnp.dot(_unpack(tab_ref[half]), _load_bf16(kvb_ref, (l,), chunk(c)),
                                preferred_element_type=_F32)
                    for j in range(npc // 2):
                        xs[l, half * npc // 2 + j, p0 + c] = x[16 * j:16 * j + 16]
                yield 2
            marks.add(str(l))

        xi = [p0 + NC - 1 - e if e < sure else jnp.where(p0 + NC - 1 >= e, p0 + NC - 1 - e, nchunks)
              for e in range(nq)]
        hi = [m if m < sure else jnp.where(m < p0 + NC, m, nchunks) for m in range(nq)]
        held = []

        def mac(l, i):
            xv = {}
            cost = 0
            acc = [None] * NC
            for m in reversed(range(nq)):
                hk = [hs[l, i, hi[m], j * PIECE:(j + 1) * PIECE] for j in range(3)]
                for c in range(NC):
                    e = m + NC - 1 - c
                    if e >= nq:
                        continue
                    if e not in xv:
                        a, b = xs[l, i, xi[e], 0:PIECE], xs[l, i, xi[e], PIECE:2 * PIECE]
                        xv[e] = (a + b, a, b)
                    new = [x * h for x, h in zip(xv[e], hk)]
                    acc[c] = new if acc[c] is None else [s + t for s, t in zip(acc[c], new)]
                    cost += 6
                cost += 1
                if m % 2 == 0:
                    if held:
                        hs[l, i, zh + nchunks + 1, 0:PIECE] = held.pop()
                    held.append(acc[NC - 1][2])
                if m % 1 == 0:
                    yield cost
                    cost = 0
            for c in range(NC):
                s1, s2, s3 = acc[c]
                z = jnp.concatenate([s1 - s3, s1 + s2], axis=0)
                mix_ref[za + nf + c * nd + l, 2 * i * PIECE:2 * (i + 1) * PIECE, :] = z.astype(_BF16)
            yield 3 * NC

        def vpu_stream():
            nln = R // LNR
            if first:
                yield "pause"
                assert "kvh" in marks
                wait(kvh_copies(0))
            for l in range(nd):
                yield from gated_kv(l)
                yield "kv%d" % l
            for l in range(nd):
                yield "wait%d" % l
                for i in range(npc):
                    yield from mac(l, i)
                    if first:
                        xs[l, i, nchunks] = jnp.zeros((2 * PIECE, T), _F32)
                        hs[l, i, nchunks] = jnp.zeros((3 * PIECE, T), _F32)
                        continue
                    k0, k1 = (40, 80)
                    k = min(max(l * npc + i, k0), k1) - k0
                    kn = min(max(l * npc + i + 1, k0), k1) - k0
                    for t in range(k * nln // (k1 - k0), kn * nln // (k1 - k0)):
                        if 1:
                            yield from layer_norm(step + 1, t)
                yield "mac%d" % l
            if first:
                yield "waitq1"
                for t in range(nln):
                    for cost in layer_norm(1, t):
                        yield cost * 3

        vpu_total = 30 * R // 8 + nd * npc * (6 * (NC * nq - NC * (NC - 1) // 2) + nq + 3 * NC)

        def mlp_in(j, c, defer=None):
            fl = tile(j)
            if first and c == 0 and j in W1_CUTS:
                n = W1_CUTS.index(j)
                wait(w1_copies(n))
                if n == 0:
                    start(kvh_copies(0))
                    marks.add("kvh")
                left = len(W1_CUTS) - 2 - n
                start(w1_copies(n + 2) if left > 1 else w2_copy(0) if left else w2_copy(1) + w2_copy(2))
            h = b1v_ref[0:1, fl]
            for kt in range(nd):
                h = h + lax.dot_general(_load_bf16(xnb_ref, (slot, kt), chunk(c)), weight_tile(w1_ref, kt, j),
                                        _NT, preferred_element_type=_F32)
                if kt < nd - 1:
                    yield w_in
            inner = h * (0.7978845608028654 + 0.035677408136300125 * (h * h))
            act = (h * (1.0 + jnp.tanh(inner))).astype(_BF16)

            def store():
                mix_ref[zb + j, chunk(c), 0:fl.stop - fl.start] = act

            if defer is None:
                store()
            else:
                defer.append(store)
            yield w_in

        hist = []

        def gated_conv(l, c):
            g = jnp.concatenate([tab_ref[2], tab_ref[3]], axis=1)
            y2 = jnp.dot(_unpack(g), _load_bf16(mix_ref, (za + nf + c * nd + l,), slice(0, 2 * C)), preferred_element_type=_F32)
            return xn_ref[slot, l, c * C:(c + 1) * C, :] * y2 + vec_ref[ks + 1:ks + 2, tile(l)]

        def finish(l, c, acc):
            rows, lanes = slice(c * C, (c + 1) * C), tile(l)
            o_ref[rows, lanes] = (0.5 * acc + q_ref[step % 3, rows, lanes].astype(_F32)).astype(o_ref.dtype)

        def mlp_out(l, c, defer):
            acc = None
            if not late:
                yield "mac%d" % l
                acc = gated_conv(l, c)
                yield 2
            for j in range(nf):
                act = _load_bf16(mix_ref, (zo[l] + j,), chunk(c), slice(0, tile(j).stop - tile(j).start))
                part = jnp.dot(act, weight_tile(w2_ref, l, j), preferred_element_type=_F32)
                acc = part if acc is None else acc + part
                hist.append(acc[0:16])
                if len(hist) > 8 and len(hist) % 4 == 0:
                    mix_ref[za + nf + NC * nd, 0:16] = hist[-9].astype(_BF16)
                if j == 3:
                    while defer:
                        defer.pop()()
                yield w_out
            if late:
                yield "mac%d" % l
                acc = acc + gated_conv(l, c)
            finish(l, c, acc)
            if late:
                yield 2

        def mlp_stream():
            defer = []
            if last_step < nsteps - 1 and 1 == 0:
                refill()
            for j in range(nf):
                for c in range(NC):
                    yield from mlp_in(j, c, defer if (j, c) == (nf - 1, NC - 1) else None)
            if last_step < nsteps - 1 and 1 == 1:
                refill()
            for l in range(nd):
                if first and l == 0:
                    wait(w2_copy(0) + w2_copy(1))
                    start(q_copy(1) + w2_copy(3))
                elif first and l == 2:
                    wait(w2_copy(2) + w2_copy(3) + q_copy(1))
                    marks.add("q1")
                    start(sum((w2_copy(m) for m in range(4, nd)), []) + kvh_copies(1))
                elif first and l >= 4:
                    wait(w2_copy(l))
                    if l == 4:
                        start(q_copy(2))
                for c in range(NC):
                    yield from mlp_out(l, c, defer)

        mxu_total = span * (NC * nf * nd * (w_in + w_out) + NC * 6 * nd)
        vpu, mlp = vpu_stream(), mlp_stream()
        marks = set()
        st = dict(n=0, done=0, seen=0, side=None, blocked=None, pause=0)

        def mxu_tick():
            st["n"] += 1
            if st["side"] is not None and st["n"] % 1 == 0:
                item = next(st["side"], None)
                if item is not None:
                    return item
                st["side"] = None
            item = next(mlp, None)
            while isinstance(item, str):
                while item not in marks:
                    if not vpu_tick():
                        for _ in st["side"]:
                            pass
                item = next(mlp, None)
            return item

        def vpu_tick():
            if st["n"] < st["pause"]:
                return False
            if st["blocked"] is not None:
                if st["blocked"] not in marks:
                    return False
                st["blocked"] = None
            got = next(vpu, None)
            if got is None:
                return False
            if not isinstance(got, str):
                st["done"] += got
            elif got == "pause":
                st["pause"] = 50
            elif got.startswith("kv"):
                st["side"] = itertools.chain(st["side"] or (), forward(int(got[2:])))
            elif got.startswith("wait"):
                st["blocked"] = got[4:]
            else:
                marks.add(got)
            return True

        while True:
            item = mxu_tick()
            if item is None:
                break
            st["seen"] += item
            while st["done"] * mxu_total < st["seen"] * vpu_total * (1 + w_kv) and vpu_tick():
                pass
        while vpu_tick():
            pass

    for variant in VARIANTS:
        pl.when((step >= variant[0]) & (step <= variant[1]))(functools.partial(body, *variant))


@jax.jit
def pallas_parallel_sum__ssm_conv_h3__dense_activation_gelu__prompt_kernel(
    A_q: jax.Array,
    A_k: jax.Array,
    A_v: jax.Array,
    A_shift_k: jax.Array,
    A_ssm_k: jax.Array,
    A_ssm_D: jax.Array,
    B_x: jax.Array,
    B_w1: jax.Array,
    B_b1: jax.Array,
    B_w2: jax.Array,
    B_b2: jax.Array,
):
    del B_x
    B, S, D = A_q.shape
    Fdim = B_w1.shape[1]
    ks = A_shift_k.shape[1]
    nsteps = S // R
    P = S // C
    nd = D // T
    assert B == 1 and S % R == 0 and D % T == 0 and ks + 2 <= 8 and nd > 4 and W1_CUTS[-1] == pl.cdiv(Fdim, T)

    args = (A_q, A_k, A_v,
            A_shift_k.T,
            A_ssm_k, A_ssm_D,
            B_w1.T,
            B_b1, B_w2, B_b2, jnp.asarray(_TABLES))
    return pl.pallas_call(
        functools.partial(_kernel, nsteps=nsteps),
        grid=(nsteps,),
        in_specs=[pl.BlockSpec(memory_space=pl.ANY)] * len(args),
        out_specs=pl.BlockSpec((None, R, D), lambda i: (0, i, 0)),
        out_shape=jax.ShapeDtypeStruct((B, S, D), A_q.dtype),
        scratch_shapes=[
            pltpu.VMEM((3, R, D), A_q.dtype),
            pltpu.VMEM((2, R, D), A_k.dtype),
            pltpu.VMEM((2, R, D), A_v.dtype),
            pltpu.VMEM((2, D, R), _BF16),
            pltpu.VMEM((nd, Fdim, T), _BF16),
            pltpu.VMEM((nd, Fdim, T), _BF16),
            pltpu.VMEM(_TABLES.shape, _U32),
            pltpu.VMEM((ks, D), A_shift_k.dtype),
            pltpu.VMEM((D,), A_ssm_D.dtype),
            pltpu.VMEM((Fdim,), B_b1.dtype),
            pltpu.VMEM((D,), B_b2.dtype),
            pltpu.SemaphoreType.DMA((4, 2)),
            pltpu.SemaphoreType.DMA((2, max(nd, len(W1_CUTS)))),
            pltpu.SemaphoreType.DMA((5,)),
            pltpu.VMEM((8, D), _F32),
            pltpu.VMEM((8, Fdim), _F32),
            pltpu.VMEM((nd, HALO + R, T), _F32),
            pltpu.VMEM((nd, C // PIECE, P + 1, 2 * PIECE, T), _F32),
            pltpu.VMEM((nd, C // PIECE, P + 2, 3 * PIECE, T), _F32),
            pltpu.VMEM((nd, 2 * C, T), _F32),
            pltpu.VMEM((2, nd, R, T), _F32),
            pltpu.VMEM((2, nd, R, T), _BF16),
            pltpu.VMEM((nd, R, T), _BF16),
            pltpu.VMEM((pl.cdiv(Fdim, T) + NC * nd + 1, max(2 * C, R), T), _BF16),
        ],
        compiler_params=pltpu.CompilerParams(
            dimension_semantics=("arbitrary",),
            vmem_limit_bytes=100 * 1024 * 1024,
        ),
    )(*args)
```

```python
import functools
import itertools
import jax
import jax.numpy as jnp
import numpy as np
from jax import lax
import jax.experimental.pallas as pl
import jax.experimental.pallas.tpu as pltpu

T = 128
C = 128
Q = C // 2
R = 256
NC = R // C
W1_CUTS = (0, 2, 5, 8, 14)
HALO = 8
PIECE = 8
KVR = 64
LNR = 64
VARIANTS = (
    (0, 0, 2, 3, 0.3, 1.0, False),
    (1, 3, 2, 3, 0.1, 0.95, True),
    (4, 5, 2, 3, 0.1, 0.95, True),
    (6, 7, 2, 3, 0.1, 0.95, True),
)

_NT = (((1,), (1,)), ((), ()))
_F32 = jnp.float32
_BF16 = jnp.bfloat16
_U32 = jnp.uint32


def _dft_tables():
    i = np.arange(C)
    f = np.where(i < Q, 2 * i, 2 * (i - Q) + 1)
    ang = np.pi * (2 * f[:, None] + 1) * i[None, :] / (2 * C)
    both = np.stack([np.cos(ang), -np.sin(ang)])
    fwd = both.reshape(2, C // PIECE, PIECE, C).transpose(1, 0, 2, 3).reshape(2 * C, C)
    inv = fwd.T * (2.0 / C)

    def words(m):
        u = np.ascontiguousarray(m, np.float32).view(np.uint32)
        u = (u + 0x7FFF + ((u >> 16) & 1)) >> 16
        return (u[0::2] | (u[1::2] << 16)).astype(np.uint32)

    inv = words(inv)
    return np.concatenate([words(fwd), inv[:, :T], inv[:, T:]]).reshape(4, Q, T)


_TABLES = _dft_tables()


def _unpack(x):
    return pltpu.bitcast(x, _BF16)


def _load_bf16(ref, lead, rows, cols=slice(None)):
    return _unpack(ref.bitcast(_U32)[(*lead, slice(rows.start // 2, rows.stop // 2), cols)])


def _kernel(q_hbm, k_hbm, v_hbm, sk_hbm, h_hbm, d_hbm, w1_hbm, b1_hbm, w2_hbm, b2_hbm, tab_hbm, o_ref,
            q_ref, k_ref, v_ref, h_ref, w1_ref, w2_ref, tab_ref, sk_ref, d_ref, b1_ref, b2_ref,
            blk_sems, w_sems, small_sems,
            vec_ref, b1v_ref, kbuf, xs, hs, kprev, xn_ref, xnb_ref, kvb_ref, mix_ref, *, nsteps):
    step = pl.program_id(0)
    D = k_hbm.shape[-1]
    Fdim = w1_hbm.shape[0]
    ks = sk_hbm.shape[0]
    nd = D // T
    nf = pl.cdiv(Fdim, T)
    npc = C // PIECE
    nchunks = nsteps * NC

    def tile(i):
        return slice(i * T, min((i + 1) * T, Fdim))

    def chunk(c):
        return slice(c * C, (c + 1) * C)

    def rows_of(s):
        return pl.ds(s * R, R) if isinstance(s, int) else pl.ds(pl.multiple_of(s * R, R), R)

    def q_copy(s):
        return [pltpu.make_async_copy(q_hbm.at[0, rows_of(s)], q_ref.at[s % 3], blk_sems.at[0, s % 2])]

    def kvh_copies(s):
        return [pltpu.make_async_copy(h_hbm.at[:, rows_of(s)], h_ref.at[s % 2], blk_sems.at[1, s % 2]),
                pltpu.make_async_copy(k_hbm.at[0, rows_of(s)], k_ref.at[s % 2], blk_sems.at[2, s % 2]),
                pltpu.make_async_copy(v_hbm.at[0, rows_of(s)], v_ref.at[s % 2], blk_sems.at[3, s % 2])]

    def w1_copies(n):
        rows = pl.ds(W1_CUTS[n] * T, min(W1_CUTS[n + 1] * T, Fdim) - W1_CUTS[n] * T)
        return [pltpu.make_async_copy(w1_hbm.at[rows, tile(l)], w1_ref.at[l, rows],
                                      w_sems.at[0, n]) for l in range(nd)]

    def w2_copy(l):
        return [pltpu.make_async_copy(w2_hbm.at[:, tile(l)], w2_ref.at[l], w_sems.at[1, l])]

    def small_copies():
        pairs = ((tab_hbm, tab_ref), (sk_hbm, sk_ref), (d_hbm, d_ref), (b1_hbm, b1_ref), (b2_hbm, b2_ref))
        return [pltpu.make_async_copy(a, b, small_sems.at[i]) for i, (a, b) in enumerate(pairs)]

    def start(copies):
        for cp in copies:
            cp.start()

    def wait(copies):
        for cp in copies:
            cp.wait()

    def weight_tile(ref, l, j):
        return _load_bf16(ref, (l,), tile(j))

    def layer_norm(s, i):
        rows = slice(i * LNR, (i + 1) * LNR)
        x = q_ref[s % 3, rows, :].astype(_F32)
        mu = jnp.mean(x, axis=-1, keepdims=True)
        yield 6 * LNR // 8
        xc = x - mu
        var = jnp.mean(xc * xc, axis=-1, keepdims=True)
        yield 14 * LNR // 8
        xn = xc * lax.rsqrt(var + 1e-5)
        for l in range(nd):
            xn_ref[s % 2, l, rows, :] = xn[:, tile(l)]
            xnb_ref[s % 2, l, rows, :] = xn[:, tile(l)].astype(_BF16)
        yield 10 * LNR // 8

    def init():
        start(q_copy(0) + small_copies() + w1_copies(0))
        wait(q_copy(0))
        start(w1_copies(1))
        for i in range(R // LNR):
            for _ in layer_norm(0, i):
                pass
        wait(small_copies())
        vec_ref[0:ks, :] = sk_ref[...].astype(_F32)
        vec_ref[ks:ks + 1, :] = d_ref[...].astype(_F32)[None, :]
        vec_ref[ks + 1:ks + 2, :] = 2.0 * b2_ref[...].astype(_F32)[None, :]
        b1v_ref[0:1, :] = b1_ref[...].astype(_F32)[None, :]
        kbuf[:, 0:HALO, :] = jnp.zeros((nd, HALO, T), _F32)

    pl.when(step == 0)(init)

    def body(first_step, last_step, w_in, w_out, w_kv, span, late):
        first = first_step == 0
        slot = step % 2
        p0 = step * NC
        nq = (last_step + 1) * NC
        sure = (first_step + 1) * NC
        za, zb, zh = step >> 12, step >> 13, step >> 14
        zo = [step >> (15 + l) for l in range(nd)]

        def refill():
            if not first:
                start(kvh_copies(step + 1) + q_copy(step + 2))

        if last_step == nsteps - 1:
            wait(kvh_copies(step))

            @pl.when(step < last_step)
            def _():
                wait(q_copy(last_step))
                start(kvh_copies(last_step))
        elif not first:
            wait(kvh_copies(step) + q_copy(step + 1))

        def gated_kv(l):
            lanes = tile(l)
            for c in range(NC):
                rows = slice(c * C, (c + 1) * C)
                kbuf[l, HALO + c * C:HALO + (c + 1) * C, :] = k_ref[slot, rows, lanes].astype(_F32)
            for c in range(NC):
                for r in range(0, C, KVR):
                    lo = c * C + r
                    ksh = None
                    for j in range(ks):
                        t = kbuf[l, HALO - j + lo:HALO - j + lo + KVR, :] * vec_ref[j:j + 1, lanes]
                        ksh = t if ksh is None else ksh + t
                    kv = ksh * v_ref[slot, lo:lo + KVR, lanes].astype(_F32)
                    kvb_ref[l, lo:lo + KVR, :] = kv.astype(_BF16)
                    yield int(w_kv * vpu_total / (nd * R // KVR))
            kbuf[l, 0:HALO, :] = kbuf[l, R:R + HALO, :]

        def forward(l):
            for half in range(2):
                kk = [lax.dot_general(_unpack(tab_ref[half]), h_ref[slot, tile(l), c * C:(c + 1) * C], _NT,
                                      preferred_element_type=_F32) for c in range(NC)]
                for j in range(npc // 2):
                    i = half * npc // 2 + j
                    prev = None if first else (kprev[l, 16 * i:16 * i + 8], kprev[l, 16 * i + 8:16 * i + 16])
                    for c in range(NC):
                        re, im = kk[c][16 * j:16 * j + 8], kk[c][16 * j + 8:16 * j + 16]
                        if prev is None:
                            re = re + vec_ref[ks:ks + 1, tile(l)]
                            hc, hd = re, im
                        elif half == 0:
                            hc, hd = re - prev[1], im + prev[0]
                        else:
                            hc, hd = re + prev[1], im - prev[0]
                        hs[l, i, p0 + c, 0:8] = hc
                        hs[l, i, p0 + c, 8:16] = hd - hc
                        hs[l, i, p0 + c, 16:24] = hd + hc
                        prev = re, im
                    kprev[l, 16 * i:16 * i + 8] = prev[0]
                    kprev[l, 16 * i + 8:16 * i + 16] = prev[1]
                yield NC
            for c in range(NC):
                for half in range(2):
                    x = jnp.dot(_unpack(tab_ref[half]), _load_bf16(kvb_ref, (l,), chunk(c)),
                                preferred_element_type=_F32)
                    for j in range(npc // 2):
                        xs[l, half * npc // 2 + j, p0 + c] = x[16 * j:16 * j + 16]
                yield 2
            marks.add(str(l))

        xi = [p0 + NC - 1 - e if e < sure else jnp.where(p0 + NC - 1 >= e, p0 + NC - 1 - e, nchunks)
              for e in range(nq)]
        hi = [m if m < sure else jnp.where(m < p0 + NC, m, nchunks) for m in range(nq)]
        held = []

        def mac(l, i):
            xv = {}
            cost = 0
            acc = [None] * NC
            for m in reversed(range(nq)):
                hk = [hs[l, i, hi[m], j * PIECE:(j + 1) * PIECE] for j in range(3)]
                for c in range(NC):
                    e = m + NC - 1 - c
                    if e >= nq:
                        continue
                    if e not in xv:
                        a, b = xs[l, i, xi[e], 0:PIECE], xs[l, i, xi[e], PIECE:2 * PIECE]
                        xv[e] = (a + b, a, b)
                    new = [x * h for x, h in zip(xv[e], hk)]
                    acc[c] = new if acc[c] is None else [s + t for s, t in zip(acc[c], new)]
                    cost += 6
                cost += 1
                if m % 2 == 0:
                    if held:
                        hs[l, i, zh + nchunks + 1, 0:PIECE] = held.pop()
                    held.append(acc[NC - 1][2])
                yield cost
                cost = 0
            for c in range(NC):
                s1, s2, s3 = acc[c]
                z = jnp.concatenate([s1 - s3, s1 + s2], axis=0)
                mix_ref[za + nf + c * nd + l, 2 * i * PIECE:2 * (i + 1) * PIECE, :] = z.astype(_BF16)
            yield 3 * NC

        def vpu_stream():
            nln = R // LNR
            if first:
                yield "pause"
                assert "kvh" in marks
                wait(kvh_copies(0))
            for l in range(nd):
                yield from gated_kv(l)
                yield "kv%d" % l
            for l in range(nd):
                yield "wait%d" % l
                for i in range(npc):
                    yield from mac(l, i)
                    if first:
                        xs[l, i, nchunks] = jnp.zeros((2 * PIECE, T), _F32)
                        hs[l, i, nchunks] = jnp.zeros((3 * PIECE, T), _F32)
                        continue
                    k0, k1 = nd * npc // 2, nd * npc
                    k = min(max(l * npc + i, k0), k1) - k0
                    kn = min(max(l * npc + i + 1, k0), k1) - k0
                    for t in range(k * nln // (k1 - k0), kn * nln // (k1 - k0)):
                        yield from layer_norm(step + 1, t)
                yield "mac%d" % l
            if first:
                yield "waitq1"
                for t in range(nln):
                    for cost in layer_norm(1, t):
                        yield cost * 3

        vpu_total = 30 * R // 8 + nd * npc * (6 * (NC * nq - NC * (NC - 1) // 2) + nq + 3 * NC)

        def mlp_in(j, c, defer=None):
            fl = tile(j)
            if first and c == 0 and j in W1_CUTS:
                n = W1_CUTS.index(j)
                wait(w1_copies(n))
                if n == 0:
                    start(kvh_copies(0))
                    marks.add("kvh")
                left = len(W1_CUTS) - 2 - n
                start(w1_copies(n + 2) if left > 1 else w2_copy(0) if left else w2_copy(1) + w2_copy(2))
            h = b1v_ref[0:1, fl]
            for kt in range(nd):
                h = h + lax.dot_general(_load_bf16(xnb_ref, (slot, kt), chunk(c)), weight_tile(w1_ref, kt, j),
                                        _NT, preferred_element_type=_F32)
                if kt < nd - 1:
                    yield w_in
            inner = h * (0.7978845608028654 + 0.035677408136300125 * (h * h))
            act = (h * (1.0 + jnp.tanh(inner))).astype(_BF16)

            def store():
                mix_ref[zb + j, chunk(c), 0:fl.stop - fl.start] = act

            if defer is None:
                store()
            else:
                defer.append(store)
            yield w_in

        hist = []

        def gated_conv(l, c):
            g = jnp.concatenate([tab_ref[2], tab_ref[3]], axis=1)
            y2 = jnp.dot(_unpack(g), _load_bf16(mix_ref, (za + nf + c * nd + l,), slice(0, 2 * C)), preferred_element_type=_F32)
            return xn_ref[slot, l, c * C:(c + 1) * C, :] * y2 + vec_ref[ks + 1:ks + 2, tile(l)]

        def finish(l, c, acc):
            rows, lanes = slice(c * C, (c + 1) * C), tile(l)
            o_ref[rows, lanes] = (0.5 * acc + q_ref[step % 3, rows, lanes].astype(_F32)).astype(o_ref.dtype)

        def mlp_out(l, c, defer):
            acc = None
            if not late:
                yield "mac%d" % l
                acc = gated_conv(l, c)
                yield 2
            for j in range(nf):
                act = _load_bf16(mix_ref, (zo[l] + j,), chunk(c), slice(0, tile(j).stop - tile(j).start))
                part = jnp.dot(act, weight_tile(w2_ref, l, j), preferred_element_type=_F32)
                acc = part if acc is None else acc + part
                hist.append(acc[0:16])
                if len(hist) > 8 and len(hist) % 4 == 0:
                    mix_ref[za + nf + NC * nd, 0:16] = hist[-9].astype(_BF16)
                if j == 3:
                    while defer:
                        defer.pop()()
                yield w_out
            if late:
                yield "mac%d" % l
                acc = acc + gated_conv(l, c)
            finish(l, c, acc)
            if late:
                yield 2

        def mlp_stream():
            defer = []
            for j in range(nf):
                for c in range(NC):
                    yield from mlp_in(j, c, defer if (j, c) == (nf - 1, NC - 1) else None)
            if last_step < nsteps - 1:
                refill()
            for l in range(nd):
                if first and l == 0:
                    wait(w2_copy(0) + w2_copy(1))
                    start(q_copy(1) + w2_copy(3))
                elif first and l == 2:
                    wait(w2_copy(2) + w2_copy(3) + q_copy(1))
                    marks.add("q1")
                    start(sum((w2_copy(m) for m in range(4, nd)), []) + kvh_copies(1))
                elif first and l >= 4:
                    wait(w2_copy(l))
                    if l == 4:
                        start(q_copy(2))
                for c in range(NC):
                    yield from mlp_out(l, c, defer)

        mxu_total = span * (NC * nf * nd * (w_in + w_out) + NC * 6 * nd)
        vpu, mlp = vpu_stream(), mlp_stream()
        marks = set()
        st = dict(n=0, done=0, seen=0, side=None, blocked=None, pause=0)

        def mxu_tick():
            st["n"] += 1
            if st["side"] is not None:
                item = next(st["side"], None)
                if item is not None:
                    return item
                st["side"] = None
            item = next(mlp, None)
            while isinstance(item, str):
                while item not in marks:
                    if not vpu_tick():
                        for _ in st["side"]:
                            pass
                item = next(mlp, None)
            return item

        def vpu_tick():
            if st["n"] < st["pause"]:
                return False
            if st["blocked"] is not None:
                if st["blocked"] not in marks:
                    return False
                st["blocked"] = None
            got = next(vpu, None)
            if got is None:
                return False
            if not isinstance(got, str):
                st["done"] += got
            elif got == "pause":
                st["pause"] = 50
            elif got.startswith("kv"):
                st["side"] = itertools.chain(st["side"] or (), forward(int(got[2:])))
            elif got.startswith("wait"):
                st["blocked"] = got[4:]
            else:
                marks.add(got)
            return True

        while True:
            item = mxu_tick()
            if item is None:
                break
            st["seen"] += item
            while st["done"] * mxu_total < st["seen"] * vpu_total * (1 + w_kv) and vpu_tick():
                pass
        while vpu_tick():
            pass

    for variant in VARIANTS:
        pl.when((step >= variant[0]) & (step <= variant[1]))(functools.partial(body, *variant))


@jax.jit
def pallas_parallel_sum__ssm_conv_h3__dense_activation_gelu__prompt_kernel(
    A_q: jax.Array,
    A_k: jax.Array,
    A_v: jax.Array,
    A_shift_k: jax.Array,
    A_ssm_k: jax.Array,
    A_ssm_D: jax.Array,
    B_x: jax.Array,
    B_w1: jax.Array,
    B_b1: jax.Array,
    B_w2: jax.Array,
    B_b2: jax.Array,
):
    del B_x
    B, S, D = A_q.shape
    Fdim = B_w1.shape[1]
    ks = A_shift_k.shape[1]
    nsteps = S // R
    P = S // C
    nd = D // T
    assert B == 1 and S % R == 0 and D % T == 0 and ks + 2 <= 8 and nd > 4 and W1_CUTS[-1] == pl.cdiv(Fdim, T)

    args = (A_q, A_k, A_v,
            A_shift_k.T,
            A_ssm_k, A_ssm_D,
            B_w1.T,
            B_b1, B_w2, B_b2, jnp.asarray(_TABLES))
    return pl.pallas_call(
        functools.partial(_kernel, nsteps=nsteps),
        grid=(nsteps,),
        in_specs=[pl.BlockSpec(memory_space=pl.ANY)] * len(args),
        out_specs=pl.BlockSpec((None, R, D), lambda i: (0, i, 0)),
        out_shape=jax.ShapeDtypeStruct((B, S, D), A_q.dtype),
        scratch_shapes=[
            pltpu.VMEM((3, R, D), A_q.dtype),
            pltpu.VMEM((2, R, D), A_k.dtype),
            pltpu.VMEM((2, R, D), A_v.dtype),
            pltpu.VMEM((2, D, R), _BF16),
            pltpu.VMEM((nd, Fdim, T), _BF16),
            pltpu.VMEM((nd, Fdim, T), _BF16),
            pltpu.VMEM(_TABLES.shape, _U32),
            pltpu.VMEM((ks, D), A_shift_k.dtype),
            pltpu.VMEM((D,), A_ssm_D.dtype),
            pltpu.VMEM((Fdim,), B_b1.dtype),
            pltpu.VMEM((D,), B_b2.dtype),
            pltpu.SemaphoreType.DMA((4, 2)),
            pltpu.SemaphoreType.DMA((2, max(nd, len(W1_CUTS)))),
            pltpu.SemaphoreType.DMA((5,)),
            pltpu.VMEM((8, D), _F32),
            pltpu.VMEM((8, Fdim), _F32),
            pltpu.VMEM((nd, HALO + R, T), _F32),
            pltpu.VMEM((nd, C // PIECE, P + 1, 2 * PIECE, T), _F32),
            pltpu.VMEM((nd, C // PIECE, P + 2, 3 * PIECE, T), _F32),
            pltpu.VMEM((nd, 2 * C, T), _F32),
            pltpu.VMEM((2, nd, R, T), _F32),
            pltpu.VMEM((2, nd, R, T), _BF16),
            pltpu.VMEM((nd, R, T), _BF16),
            pltpu.VMEM((pl.cdiv(Fdim, T) + NC * nd + 1, max(2 * C, R), T), _BF16),
        ],
        compiler_params=pltpu.CompilerParams(
            dimension_semantics=("arbitrary",),
            vmem_limit_bytes=100 * 1024 * 1024,
        ),
    )(*args)
```

```python
import functools
import itertools
import jax
import jax.numpy as jnp
import numpy as np
from jax import lax
import jax.experimental.pallas as pl
import jax.experimental.pallas.tpu as pltpu

T = 128
C = 128
Q = C // 2
R = 256
NC = R // C
W1_CUTS = (0, 4, 10, 14)
FIRST_INIT = ("q0 a0", "x0")
FIRST_IN = (("a0", "a1"), ("a1", "b0"), ("a2", "b1 b2"))
FIRST_KV = ("x0", "a2")
FIRST_OUT = (("b0", "b3 b4 q1"), ("b1 b2", "x1"), ("", "q2"), ("b3 b4 q1", ""), ("", ""))
HALO = 8
PIECE = 8
KVR = 128
LNR = 64
VARIANTS = (
    (0, 0, 2, 3, 0.15, 1.0, False),
    (1, 2, 2, 3, 0.1, 0.95, True),
    (3, 4, 2, 3, 0.1, 0.95, True),
    (5, 6, 2, 3, 0.1, 0.95, True),
    (7, 7, 2, 3, 0.1, 0.95, True),
)

_NT = (((1,), (1,)), ((), ()))
_F32 = jnp.float32
_BF16 = jnp.bfloat16
_U32 = jnp.uint32


def _dft_tables():
    i = np.arange(C)
    f = np.where(i < Q, 2 * i, 2 * (i - Q) + 1)
    ang = np.pi * (2 * f[:, None] + 1) * i[None, :] / (2 * C)
    both = np.stack([np.cos(ang), -np.sin(ang)])
    fwd = both.reshape(2, C // PIECE, PIECE, C).transpose(1, 0, 2, 3).reshape(2 * C, C)
    inv = fwd.T * (2.0 / C)

    def words(m):
        u = np.ascontiguousarray(m, np.float32).view(np.uint32)
        u = (u + 0x7FFF + ((u >> 16) & 1)) >> 16
        return (u[0::2] | (u[1::2] << 16)).astype(np.uint32)

    inv = words(inv)
    return np.concatenate([words(fwd), inv[:, :T], inv[:, T:]]).reshape(4, Q, T)


_TABLES = _dft_tables()


def _unpack(x):
    return pltpu.bitcast(x, _BF16)


def _load_bf16(ref, lead, rows, cols=slice(None)):
    return _unpack(ref.bitcast(_U32)[(*lead, slice(rows.start // 2, rows.stop // 2), cols)])


def _kernel(q_hbm, k_hbm, v_hbm, sk_hbm, h_hbm, d_hbm, w1_hbm, b1_hbm, w2_hbm, b2_hbm, tab_hbm, o_ref,
            q_ref, k_ref, v_ref, h_ref, w1_ref, w2_ref, tab_ref, sk_ref, d_ref, b1_ref, b2_ref,
            blk_sems, w_sems, small_sems,
            vec_ref, b1v_ref, kbuf, xs, hs, kprev, xn_ref, xnb_ref, kvb_ref, mix_ref, zeros_ref, *, nsteps):
    step = pl.program_id(0)
    D = k_hbm.shape[-1]
    Fdim = w1_hbm.shape[0]
    ks = sk_hbm.shape[0]
    nd = D // T
    nf = pl.cdiv(Fdim, T)
    npc = C // PIECE
    nchunks = nsteps * NC

    def tile(i):
        return slice(i * T, min((i + 1) * T, Fdim))

    def chunk(c):
        return slice(c * C, (c + 1) * C)

    def rows_of(s):
        return pl.ds(s * R, R) if isinstance(s, int) else pl.ds(pl.multiple_of(s * R, R), R)

    def q_copy(s):
        return [pltpu.make_async_copy(q_hbm.at[0, rows_of(s)], q_ref.at[s % 3], blk_sems.at[0, s % 2])]

    def kvh_copies(s):
        return [pltpu.make_async_copy(h_hbm.at[:, rows_of(s)], h_ref.at[s % 2], blk_sems.at[1, s % 2]),
                pltpu.make_async_copy(k_hbm.at[0, rows_of(s)], k_ref.at[s % 2], blk_sems.at[2, s % 2]),
                pltpu.make_async_copy(v_hbm.at[0, rows_of(s)], v_ref.at[s % 2], blk_sems.at[3, s % 2])]

    def w1_copies(n):
        rows = pl.ds(W1_CUTS[n] * T, min(W1_CUTS[n + 1] * T, Fdim) - W1_CUTS[n] * T)
        return [pltpu.make_async_copy(w1_hbm.at[rows, tile(l)], w1_ref.at[l, rows],
                                      w_sems.at[0, n]) for l in range(nd)]

    def w2_copy(l):
        return [pltpu.make_async_copy(w2_hbm.at[:, tile(l)], w2_ref.at[l], w_sems.at[1, l])]

    def small_copies():
        pairs = ((tab_hbm, tab_ref), (sk_hbm, sk_ref), (d_hbm, d_ref), (b1_hbm, b1_ref), (b2_hbm, b2_ref))
        return [pltpu.make_async_copy(a, b, small_sems.at[i]) for i, (a, b) in enumerate(pairs)]

    def start(copies):
        for cp in copies:
            cp.start()

    def wait(copies):
        for cp in copies:
            cp.wait()

    started = set()

    def transfer(waits, starts):
        kinds = dict(q=q_copy, x=kvh_copies, a=w1_copies, b=w2_copy)
        for name in waits.split():
            started.remove(name)
        wait([cp for name in waits.split() for cp in kinds[name[0]](int(name[1:]))])
        started.update(starts.split())
        start([cp for name in starts.split() for cp in kinds[name[0]](int(name[1:]))])

    def weight_tile(ref, l, j):
        return _load_bf16(ref, (l,), tile(j))

    def layer_norm(s, i):
        rows = slice(i * LNR, (i + 1) * LNR)
        x = q_ref[s % 3, rows, :].astype(_F32)
        mu = jnp.mean(x, axis=-1, keepdims=True)
        yield 6 * LNR // 8
        xc = x - mu
        var = jnp.mean(xc * xc, axis=-1, keepdims=True)
        yield 14 * LNR // 8
        xn = xc * lax.rsqrt(var + 1e-5)
        for l in range(nd):
            xn_ref[s % 2, l, rows, :] = xn[:, tile(l)]
            xnb_ref[s % 2, l, rows, :] = xn[:, tile(l)].astype(_BF16)
        yield 10 * LNR // 8

    def init():
        transfer("", FIRST_INIT[0])
        start(small_copies())
        for i in range(3 + nd):
            zeros_ref[i] = 0
        transfer("q0", FIRST_INIT[1])
        for i in range(R // LNR):
            for _ in layer_norm(0, i):
                pass
        wait(small_copies())
        vec_ref[0:ks, :] = sk_ref[...].astype(_F32)
        vec_ref[ks:ks + 1, :] = d_ref[...].astype(_F32)[None, :]
        vec_ref[ks + 1:ks + 2, :] = 2.0 * b2_ref[...].astype(_F32)[None, :]
        b1v_ref[0:1, :] = b1_ref[...].astype(_F32)[None, :]
        kbuf[:, 0:HALO, :] = jnp.zeros((nd, HALO, T), _F32)

    pl.when(step == 0)(init)

    def body(first_step, last_step, w_in, w_out, w_kv, span, late):
        first = first_step == 0
        slot = step % 2
        p0 = step * NC
        nq = (last_step + 1) * NC
        sure = min(first_step + 1, last_step) * NC
        za, zb, zh, *zo = [zeros_ref[i] for i in range(3 + nd)]

        last = last_step == nsteps - 1
        if not first:
            wait(kvh_copies(step) + ([] if last else q_copy(step + 1)))

        if last_step == nsteps - 2:
            pl.when(step < last_step)(lambda: start(q_copy(step + 2)))
        elif not (first or last):
            start(q_copy(step + 2))
        if not (first or last):
            start(kvh_copies(step + 1))

        def gated_kv(l):
            lanes = tile(l)
            for c in range(NC):
                rows = slice(c * C, (c + 1) * C)
                kbuf[l, HALO + c * C:HALO + (c + 1) * C, :] = k_ref[slot, rows, lanes].astype(_F32)
            for c in range(NC):
                for r in range(0, C, KVR):
                    lo = c * C + r
                    ksh = None
                    for j in range(ks):
                        t = kbuf[l, HALO - j + lo:HALO - j + lo + KVR, :] * vec_ref[j:j + 1, lanes]
                        ksh = t if ksh is None else ksh + t
                    kv = ksh * v_ref[slot, lo:lo + KVR, lanes].astype(_F32)
                    kvb_ref[l, lo:lo + KVR, :] = kv.astype(_BF16)
                    yield int(w_kv * vpu_total / (nd * R // KVR))
            kbuf[l, 0:HALO, :] = kbuf[l, R:R + HALO, :]

        def forward(l):
            for half in range(2):
                kk = [lax.dot_general(_unpack(tab_ref[half]), h_ref[slot, tile(l), c * C:(c + 1) * C], _NT,
                                      preferred_element_type=_F32) for c in range(NC)]
                for j in range(npc // 2):
                    i = half * npc // 2 + j
                    prev = None if first else (kprev[l, 16 * i:16 * i + 8], kprev[l, 16 * i + 8:16 * i + 16])
                    for c in range(NC):
                        re, im = kk[c][16 * j:16 * j + 8], kk[c][16 * j + 8:16 * j + 16]
                        if prev is None:
                            re = re + vec_ref[ks:ks + 1, tile(l)]
                            hc, hd = re, im
                        elif half == 0:
                            hc, hd = re - prev[1], im + prev[0]
                        else:
                            hc, hd = re + prev[1], im - prev[0]
                        hs[l, i, p0 + c, 0:8] = hc
                        hs[l, i, p0 + c, 8:16] = hd - hc
                        hs[l, i, p0 + c, 16:24] = hd + hc
                        prev = re, im
                    kprev[l, 16 * i:16 * i + 8] = prev[0]
                    kprev[l, 16 * i + 8:16 * i + 16] = prev[1]
                yield NC
            for c in range(NC):
                for half in range(2):
                    x = jnp.dot(_unpack(tab_ref[half]), _load_bf16(kvb_ref, (l,), chunk(c)),
                                preferred_element_type=_F32)
                    for j in range(npc // 2):
                        xs[l, half * npc // 2 + j, p0 + c] = x[16 * j:16 * j + 16]
                yield 2
            marks.add(str(l))

        xi = [p0 + NC - 1 - e if e < sure else jnp.where(p0 + NC - 1 >= e, p0 + NC - 1 - e, nchunks)
              for e in range(nq)]
        hi = [m if m < sure else jnp.where(m < p0 + NC, m, nchunks) for m in range(nq)]
        held = []

        def mac(l, i):
            xv = {}
            cost = 0
            acc = [None] * NC
            for m in reversed(range(nq)):
                hk = [hs[l, i, hi[m], j * PIECE:(j + 1) * PIECE] for j in range(3)]
                for c in range(NC):
                    e = m + NC - 1 - c
                    if e >= nq:
                        continue
                    if e not in xv:
                        a, b = xs[l, i, xi[e], 0:PIECE], xs[l, i, xi[e], PIECE:2 * PIECE]
                        xv[e] = (a + b, a, b)
                    new = [x * h for x, h in zip(xv[e], hk)]
                    acc[c] = new if acc[c] is None else [s + t for s, t in zip(acc[c], new)]
                    cost += 6
                cost += 1
                if m % 2 == 0:
                    if held:
                        hs[l, i, zh + nchunks + 1, 0:PIECE] = held.pop()
                    held.append(acc[NC - 1][2])
                yield cost
                cost = 0
            for c in range(NC):
                s1, s2, s3 = acc[c]
                z = jnp.concatenate([s1 - s3, s1 + s2], axis=0)
                mix_ref[za + nf + c * nd + l, 2 * i * PIECE:2 * (i + 1) * PIECE, :] = z.astype(_BF16)
            yield 3 * NC

        def vpu_stream():
            nln = R // LNR
            if first:
                yield "pause"
                transfer(*FIRST_KV)
            for l in range(nd):
                yield from gated_kv(l)
                yield "kv%d" % l
            for l in range(nd):
                yield "wait%d" % l
                for i in range(npc):
                    yield from mac(l, i)
                    if first:
                        xs[l, i, nchunks] = jnp.zeros((2 * PIECE, T), _F32)
                        hs[l, i, nchunks] = jnp.zeros((3 * PIECE, T), _F32)
                        continue
                    k0, k1 = nd * npc // 2, nd * npc
                    k = min(max(l * npc + i, k0), k1) - k0
                    kn = min(max(l * npc + i + 1, k0), k1) - k0
                    for t in range(k * nln // (k1 - k0), kn * nln // (k1 - k0)):
                        if not last:
                            yield from layer_norm(step + 1, t)
                yield "mac%d" % l
            if first:
                yield "waitq1"
                for t in range(nln):
                    for cost in layer_norm(step + 1, t):
                        yield cost * 3

        vpu_total = (0 if last else 30 * R // 8) + nd * npc * (6 * (NC * nq - NC * (NC - 1) // 2) + nq + 3 * NC)

        def mlp_in(j, c, defer=None):
            fl = tile(j)
            if first and c == 0 and j in W1_CUTS:
                transfer(*FIRST_IN[W1_CUTS.index(j)])
            h = b1v_ref[0:1, fl]
            for kt in range(nd):
                h = h + lax.dot_general(_load_bf16(xnb_ref, (slot, kt), chunk(c)), weight_tile(w1_ref, kt, j),
                                        _NT, preferred_element_type=_F32)
                if kt < nd - 1:
                    yield w_in
            inner = h * (0.7978845608028654 + 0.035677408136300125 * (h * h))
            act = (h * (1.0 + jnp.tanh(inner))).astype(_BF16)

            def store():
                mix_ref[zb + j, chunk(c), 0:fl.stop - fl.start] = act

            if defer is None:
                store()
            else:
                defer.append(store)
            yield w_in

        hist = []

        def gated_conv(l, c):
            g = jnp.concatenate([tab_ref[2], tab_ref[3]], axis=1)
            y2 = jnp.dot(_unpack(g), _load_bf16(mix_ref, (za + nf + c * nd + l,), slice(0, 2 * C)), preferred_element_type=_F32)
            return xn_ref[slot, l, c * C:(c + 1) * C, :] * y2 + vec_ref[ks + 1:ks + 2, tile(l)]

        def finish(l, c, acc):
            rows, lanes = slice(c * C, (c + 1) * C), tile(l)
            o_ref[rows, lanes] = (0.5 * acc + q_ref[step % 3, rows, lanes].astype(_F32)).astype(o_ref.dtype)

        def mlp_out(l, c, defer):
            acc = None
            if not late:
                yield "mac%d" % l
                acc = gated_conv(l, c)
                yield 2
            for j in range(nf):
                act = _load_bf16(mix_ref, (zo[l] + j,), chunk(c), slice(0, tile(j).stop - tile(j).start))
                part = jnp.dot(act, weight_tile(w2_ref, l, j), preferred_element_type=_F32)
                acc = part if acc is None else acc + part
                hist.append(acc[0:16])
                if len(hist) > 8 and len(hist) % 4 == 0:
                    mix_ref[za + nf + NC * nd, 0:16] = hist[-9].astype(_BF16)
                if j == 3:
                    while defer:
                        defer.pop()()
                yield w_out
            if late:
                yield "mac%d" % l
                acc = acc + gated_conv(l, c)
            finish(l, c, acc)
            if late:
                yield 2

        def mlp_stream():
            defer = []
            for j in range(nf):
                for c in range(NC):
                    yield from mlp_in(j, c, defer if (j, c) == (nf - 1, NC - 1) else None)
            for l in range(nd):
                if first:
                    transfer(*FIRST_OUT[l])
                    marks.update(FIRST_OUT[l][0].split())
                for c in range(NC):
                    yield from mlp_out(l, c, defer)

        mxu_total = span * (NC * nf * nd * (w_in + w_out) + NC * 6 * nd)
        vpu, mlp = vpu_stream(), mlp_stream()
        marks = set()
        st = dict(n=0, done=0, seen=0, side=None, blocked=None, pause=0)

        def mxu_tick():
            st["n"] += 1
            if st["side"] is not None:
                item = next(st["side"], None)
                if item is not None:
                    return item
                st["side"] = None
            item = next(mlp, None)
            while isinstance(item, str):
                while item not in marks:
                    if not vpu_tick():
                        for _ in st["side"]:
                            pass
                item = next(mlp, None)
            return item

        def vpu_tick():
            if st["n"] < st["pause"]:
                return False
            if st["blocked"] is not None:
                if st["blocked"] not in marks:
                    return False
                st["blocked"] = None
            got = next(vpu, None)
            if got is None:
                return False
            if not isinstance(got, str):
                st["done"] += got
            elif got == "pause":
                st["pause"] = 40
            elif got.startswith("kv"):
                st["side"] = itertools.chain(st["side"] or (), forward(int(got[2:])))
            elif got.startswith("wait"):
                st["blocked"] = got[4:]
            else:
                marks.add(got)
            return True

        while True:
            item = mxu_tick()
            if item is None:
                break
            st["seen"] += item
            while st["done"] * mxu_total < st["seen"] * vpu_total * (1 + w_kv) and vpu_tick():
                pass
        while vpu_tick():
            pass

    for variant in VARIANTS:
        pl.when((step >= variant[0]) & (step <= variant[1]))(functools.partial(body, *variant))


@jax.jit
def pallas_parallel_sum__ssm_conv_h3__dense_activation_gelu__prompt_kernel(
    A_q: jax.Array,
    A_k: jax.Array,
    A_v: jax.Array,
    A_shift_k: jax.Array,
    A_ssm_k: jax.Array,
    A_ssm_D: jax.Array,
    B_x: jax.Array,
    B_w1: jax.Array,
    B_b1: jax.Array,
    B_w2: jax.Array,
    B_b2: jax.Array,
):
    del B_x
    B, S, D = A_q.shape
    Fdim = B_w1.shape[1]
    ks = A_shift_k.shape[1]
    nsteps = S // R
    P = S // C
    nd = D // T
    assert B == 1 and S % R == 0 and D % T == 0 and ks + 2 <= 8 and nd == len(FIRST_OUT)
    assert tuple(VARIANTS[0][:2]) == (0, 0) and tuple(VARIANTS[-1][:2]) == (nsteps - 1, nsteps - 1) and W1_CUTS[-1] == pl.cdiv(Fdim, T)

    args = (A_q, A_k, A_v,
            A_shift_k.T,
            A_ssm_k, A_ssm_D,
            B_w1.T,
            B_b1, B_w2, B_b2, jnp.asarray(_TABLES))
    return pl.pallas_call(
        functools.partial(_kernel, nsteps=nsteps),
        grid=(nsteps,),
        in_specs=[pl.BlockSpec(memory_space=pl.ANY)] * len(args),
        out_specs=pl.BlockSpec((None, R, D), lambda i: (0, i, 0)),
        out_shape=jax.ShapeDtypeStruct((B, S, D), A_q.dtype),
        scratch_shapes=[
            pltpu.VMEM((3, R, D), A_q.dtype),
            pltpu.VMEM((2, R, D), A_k.dtype),
            pltpu.VMEM((2, R, D), A_v.dtype),
            pltpu.VMEM((2, D, R), _BF16),
            pltpu.VMEM((nd, Fdim, T), _BF16),
            pltpu.VMEM((nd, Fdim, T), _BF16),
            pltpu.VMEM(_TABLES.shape, _U32),
            pltpu.VMEM((ks, D), A_shift_k.dtype),
            pltpu.VMEM((D,), A_ssm_D.dtype),
            pltpu.VMEM((Fdim,), B_b1.dtype),
            pltpu.VMEM((D,), B_b2.dtype),
            pltpu.SemaphoreType.DMA((4, 2)),
            pltpu.SemaphoreType.DMA((2, max(nd, len(W1_CUTS)))),
            pltpu.SemaphoreType.DMA((5,)),
            pltpu.VMEM((8, D), _F32),
            pltpu.VMEM((8, Fdim), _F32),
            pltpu.VMEM((nd, HALO + R, T), _F32),
            pltpu.VMEM((nd, C // PIECE, P + 1, 2 * PIECE, T), _F32),
            pltpu.VMEM((nd, C // PIECE, P + 2, 3 * PIECE, T), _F32),
            pltpu.VMEM((nd, 2 * C, T), _F32),
            pltpu.VMEM((2, nd, R, T), _F32),
            pltpu.VMEM((2, nd, R, T), _BF16),
            pltpu.VMEM((nd, R, T), _BF16),
            pltpu.VMEM((pl.cdiv(Fdim, T) + NC * nd + 1, max(2 * C, R), T), _BF16),
            pltpu.SMEM((3 + nd,), jnp.int32),
        ],
        compiler_params=pltpu.CompilerParams(
            dimension_semantics=("arbitrary",),
            vmem_limit_bytes=100 * 1024 * 1024,
        ),
    )(*args)
```
